```python
import os as _os
_os.environ.setdefault("JAX_PLATFORMS", "cpu")
import jax
import jax.numpy as jnp

def _softmax(x, axis=-1):
    return jax.nn.softmax(x, axis=axis)
def _gelu(x):
    return jax.nn.gelu(x, approximate=True)
def _silu(x):
    return jax.nn.silu(x)
def _sigmoid(x):
    return jax.nn.sigmoid(x)
def _layernorm(x, axis=-1, eps=1e-5):
    m = jnp.mean(x, axis=axis, keepdims=True)
    v = jnp.var(x, axis=axis, keepdims=True)
    return (x - m) / jnp.sqrt(v + eps)
def _scatter_add(tgt, idx, src, axis=0):
    return tgt.at[idx].add(src)
def _segment_sum(src, seg, n):
    return jax.ops.segment_sum(src, seg, n)
class _Rng:
    def __init__(self, key):
        self._k = key
    def _next(self):
        self._k, sub = jax.random.split(self._k)
        return sub
    def normal(self, shape):
        return jax.random.normal(self._next(), shape, dtype=jnp.bfloat16)
    def randint(self, lo, hi, shape):
        return jax.random.randint(self._next(), shape, lo, hi, dtype=jnp.int32)
    def uniform(self, shape, lo=0.0, hi=1.0):
        return jax.random.uniform(self._next(), shape, jnp.bfloat16, lo, hi)
    def permutation(self, n):
        return jax.random.permutation(self._next(), n)


kernel_name = 'recurrent_scan__softmax_full_mha__glu_gated_glu__prompt'

def setup_inputs():
    _rng = _Rng(jax.random.key(int.from_bytes(__import__("os").urandom(4), "little")))
    _w = (lambda a: (lambda t: t.astype(jnp.bfloat16) if jnp.issubdtype(t.dtype, jnp.floating) else t)(jnp.asarray(a)))
    def _A_setup():
        B, S, D = 1, 2048, 1024
        return {
            "x": _w((lambda *s: _rng.normal(s) * 0.05)(B, S, D)),
            "wqkv": _w((lambda *s: _rng.normal(s) * 0.05)(D, 3 * D)),
            "wo": _w((lambda *s: _rng.normal(s) * 0.05)(D, D)),
        }
    _A_in = _A_setup()

    def _B_setup():
        B, S, D, F = 1, 2048, 1024, 3584
        return {
            "x": _w((lambda *s: _rng.normal(s) * 0.05)(B, S, D)),
            "w_gate": _w((lambda *s: _rng.normal(s) * 0.05)(D, F)),
            "w_up": _w((lambda *s: _rng.normal(s) * 0.05)(D, F)),
            "w_down": _w((lambda *s: _rng.normal(s) * 0.05)(F, D)),
        }
    _B_in = _B_setup()

    return {
        "A_x": _A_in["x"],
        "A_wqkv": _A_in["wqkv"],
        "A_wo": _A_in["wo"],
        "B_x": _B_in["x"],
        "B_w_gate": _B_in["w_gate"],
        "B_w_up": _B_in["w_up"],
        "B_w_down": _B_in["w_down"],
    }

def reference(A_x, A_wqkv, A_wo, B_x, B_w_gate, B_w_up, B_w_down):
    def _A_ref(x, wqkv, wo):
        B, S, D = x.shape
        H = 32; Dh = D // H
        qkv = (lambda x, *d: x.transpose(*d))((x @ wqkv).reshape(B, S, 3, H, Dh), 2, 0, 3, 1, 4)
        q, k, v = qkv[0], qkv[1], qkv[2]
        scale = Dh ** -0.5
        scores = jnp.einsum("bhqd,bhkd->bhqk", q, k) * scale
        p = _softmax(scores, axis=-1)
        o = jnp.einsum("bhqk,bhkd->bhqd", p, v)
        return (lambda x, *d: x.transpose(*d))(o, 0, 2, 1, 3).reshape(B, S, D) @ wo

    def _B_ref(x, w_gate, w_up, w_down):
        g = jnp.einsum("bsd,df->bsf", x, w_gate)
        u = jnp.einsum("bsd,df->bsf", x, w_up)
        h = _sigmoid(g) * u
        return jnp.einsum("bsf,fd->bsd", h, w_down)

    x = A_x
    xn = _layernorm(x, axis=-1)
    s = _A_ref(xn, A_wqkv, A_wo)
    g = _silu(_B_ref(xn, B_w_gate, B_w_up, B_w_down))
    return x + s * g
```

```python
import contextlib
import itertools
import math

import jax
import jax.numpy as jnp
from jax import lax
import jax.experimental.pallas as pl
import jax.experimental.pallas.tpu as pltpu

F32 = jnp.float32
BF16 = jnp.bfloat16
U32 = jnp.uint32

N_HEADS = 32
LN_EPS = 1e-5
LANES = 128
SPLIT = 4
N_PROD = 49
CK = 128
LAG = 2
PACE = 3
CUT = 4
FC = SPLIT * LANES
X_PIECE = 128
LN_ROWS = 16
SCOPES = False

_A_TERMS = (
    ((1, 0, 0),),
    ((1, 0, 0), (1, 0, 1)),
    ((1, 1, 0), (1, 1, 1)),
    ((1, 1, 1),),
    ((1, 0, 0), (1, 1, 1)),
    ((1, 1, 0), (-1, 0, 0)),
    ((1, 0, 1), (-1, 1, 1)),
)
_B_TERMS = (
    ((1, 0, 1), (-1, 1, 1)),
    ((1, 1, 1),),
    ((1, 0, 0),),
    ((1, 1, 0), (-1, 0, 0)),
    ((1, 0, 0), (1, 1, 1)),
    ((1, 0, 0), (1, 0, 1)),
    ((1, 1, 0), (1, 1, 1)),
)


def _scope(name):
    return jax.named_scope(name) if SCOPES else contextlib.nullcontext()


def _signed_sum(terms, block):
    acc = None
    for sign, r, c in terms:
        b = block(r, c).astype(F32)
        acc = b if acc is None else (acc + b if sign > 0 else acc - b)
    return acc


def _operand(table, i, block):
    terms = [
        (s0 * s1, 2 * r0 + r1, 2 * c0 + c1)
        for (s0, r0, c0), (s1, r1, c1) in itertools.product(table[i // 7], table[i % 7])
    ]
    if len(terms) == 1:
        return block(*terms[0][1:]).astype(BF16)
    return _signed_sum(terms, block).astype(BF16)


def _all_operands(table, block):
    for outer in table:
        half = {
            (r, c): _signed_sum(outer, lambda i, j: block(2 * i + r, 2 * j + c))
            for r in range(2)
            for c in range(2)
        }
        for inner in table:
            yield _signed_sum(inner, lambda i, j: half[i, j]).astype(BF16)


def _combine(k, v, put, get):
    if k in (0, 2, 4):
        put(k, v)
        return None
    if k == 1:
        put(1, v)
        return 0, 1, get(0) + v
    if k == 3:
        put(3, v - get(1))
        return 1, 0, get(2) + v
    if k == 5:
        return 1, 1, get(0) - get(2) + get(4) + v
    return 0, 0, get(3) + get(4) + v


def _strassen(product, emit, tmp=None):
    kept = {}

    def slots(base):
        def put(n, v):
            if tmp is None:
                kept[base + n] = v
            else:
                tmp[base + n][...] = v

        return put, lambda n: kept[base + n] if tmp is None else tmp[base + n][...]

    for i in range(N_PROD):
        inner = _combine(i % 7, product(i), *slots(0))
        if inner is not None:
            r, c, v = inner
            outer = _combine(i // 7, v, *slots(5 + 5 * (2 * r + c)))
            if outer is not None:
                emit(2 * outer[0] + r, 2 * outer[1] + c, outer[2])


def _pack(x):
    return pltpu.bitcast(x, U32)


def _unpack(x):
    return pltpu.bitcast(x, BF16)


def _dot(a, b):
    return jnp.dot(a, b, preferred_element_type=F32)


def _sigmoid(x):
    return 0.5 * jnp.tanh(0.5 * x) + 0.5


def _fold_rows(op, x):
    r = x[0:8]
    for i in range(1, x.shape[0] // 8):
        r = op(r, x[8 * i : 8 * i + 8])
    return r


def _kernel(
    x_hbm, wqkv_hbm, wo_hbm, wg_hbm, wu_hbm, wd_hbm, out_hbm,
    x_v, w_v, wo_v, wd_v, xc_v, a_v, tmp_v, zero_s,
    x_sem, wq_sem, w_sem, wo_sem, wd_sem, out_sem,
):
    S, D = x_v.shape
    n_fc = wd_v.shape[0]
    mb, kb = S // SPLIT, D // SPLIT
    dh = D // N_HEADS
    hpg = LANES // dh
    n_grp = D // LANES
    gpb = kb // LANES
    per_mat = D // FC

    def x_copy(i):
        rows = pl.ds(i * X_PIECE, X_PIECE)
        return pltpu.make_async_copy(x_hbm.at[rows], x_v.at[rows], x_sem.at[i])

    def wq_copy(c):
        cols = pl.ds(c * kb, kb)
        return pltpu.make_async_copy(wqkv_hbm.at[:, cols], wo_v.at[c], wq_sem.at[c])

    def wo_copy(c):
        cols = pl.ds(c * kb, kb)
        return pltpu.make_async_copy(wo_hbm.at[:, cols], wo_v.at[c], wo_sem.at[c])

    def w_copy(src, col, slot):
        return pltpu.make_async_copy(
            src.at[:, pl.ds(col * FC, FC)], w_v.at[slot], w_sem.at[slot]
        )

    def kv_copies():
        return [
            w_copy(wqkv_hbm, (1 + i) * per_mat + j, 2 * j + i)
            for j in range(per_mat)
            for i in range(2)
        ]

    def ffn_copies():
        return [
            copy
            for j in range(n_fc)
            for copy in (
                w_copy(wg_hbm, j, 2 * j),
                w_copy(wu_hbm, j, 2 * j + 1),
                pltpu.make_async_copy(
                    wd_hbm.at[pl.ds(j * FC, FC)], wd_v.at[j], wd_sem.at[j]
                ),
            )
        ]

    def temporaries():
        zero = zero_s[0]
        return [t.at[zero] for t in tmp_v]

    def paired_projection(j, emit, beside=None):
        def w_block(r, c):
            rows, cols = pl.ds(r * kb, kb), pl.ds(c * LANES, LANES)
            return jnp.concatenate([w_v[2 * j + i, rows, cols] for i in range(2)], 1)

        def product(i):
            result = _dot(_unpack(xc_v[i]), _operand(_B_TERMS, i, w_block))
            if beside is not None:
                beside(i)
            return result

        _strassen(product, emit, temporaries())

    def square_weight(i):
        return _operand(_B_TERMS, i, lambda r, c: wo_v[c, r * kb : (r + 1) * kb, :])

    def attention_branch(qt_v, k_v, vt_v, sc_v, carry_v, o_v):
        pieces = mb // X_PIECE
        queue = []
        for r in range(SPLIT):
            queue += [x_copy(r * pieces + i) for i in range(pieces)]
            queue.insert(len(queue) - pieces // 2, wq_copy(SPLIT - 1 - r))
        queue += kv_copies()
        started = iter(queue)
        for _ in range(IN_FLIGHT):
            next(started).start()
        zero_s[0] = 0

        def arrived(copy):
            copy.wait()
            following = next(started, None)
            if following is not None:
                following.start()

        def layernorm(r):
            for i in range(pieces):
                if i == pieces - pieces // 2:
                    arrived(wq_copy(SPLIT - 1 - r))
                arrived(x_copy(r * pieces + i))
                for row in range(i * X_PIECE, (i + 1) * X_PIECE, LN_ROWS):
                    x = x_v[pl.ds(r * mb + row, LN_ROWS), :].astype(F32)
                    x = x - jnp.mean(x, axis=-1, keepdims=True)
                    var = jnp.mean(x * x, axis=-1, keepdims=True)
                    x = x * lax.rsqrt(var + LN_EPS)
                    for c in range(SPLIT):
                        a_v[r * SPLIT + c, row : row + LN_ROWS, :] = x[
                            :, c * kb : (c + 1) * kb
                        ]

        def q_product(i):
            if i in LN_AT:
                layernorm(LN_AT.index(i))
            a = _operand(_A_TERMS, i, lambda r, c: a_v[r * SPLIT + c, 0:mb, :])
            xc_v[i] = _pack(a)
            return _dot(a, square_weight(i))

        def emit_q(r, c, v):
            t = _pack((v * (dh**-0.5 * math.log2(math.e))).astype(BF16).T)
            for g in range(gpb):
                qt_v[(c * gpb + g) * SPLIT + r] = t[g * 64 : (g + 1) * 64]

        with _scope("q"):
            _strassen(q_product, emit_q, temporaries())
            for copy in started:
                copy.start()
            for copy in kv_copies():
                copy.wait()

        @pl.loop(0, per_mat)
        def _(j):
            def emit(r, c, v):
                v = v.astype(BF16)
                g = j * SPLIT + c
                k_v[g, r * mb // 2 : (r + 1) * mb // 2, :] = _pack(v)[:, :LANES]
                vt_v[g, :, r * mb : (r + 1) * mb] = _pack(v[:, LANES:].T)

            with _scope("kv"):
                paired_projection(j, emit)

        for c in range(SPLIT):
            wo_copy(c).start()
        for copy in ffn_copies():
            copy.start()

        n_ck = S // CK
        n_step = n_grp * SPLIT

        def attend(t, lo, hi, n_units):
            queries, maxima, tops, sums, accs = {}, {}, {}, {}, {}
            top_log, sum_log, outs = [], [], []
            if lo > 0:
                maxima[0], tops[1] = carry_v[0:8], carry_v[8:16]
                sums[0], accs[0] = carry_v[16:24], carry_v[24 : 24 + dh]

            def score(u, c):
                step, h = t + u // hpg, u % hpg
                if u not in queries:
                    r0, r1 = h * dh // 2, (h + 1) * dh // 2
                    parts = [qt_v[step, r0:r1, :]]
                    if r0:
                        parts.insert(0, jnp.zeros((r0, mb), U32))
                    if r1 < LANES // 2:
                        parts.append(jnp.zeros((LANES // 2 - r1, mb), U32))
                    queries[u] = _unpack(jnp.concatenate(parts, axis=0))
                k = k_v[step // SPLIT, c * CK // 2 : (c + 1) * CK // 2, :]
                s = _dot(_unpack(k), queries[u])
                sc_v[u % 2][c * CK : (c + 1) * CK, :] = s
                top = _fold_rows(jnp.maximum, s)
                tops[u] = jnp.maximum(tops[u], top) if c else top
                top_log.append(tops[u])
                if c == n_ck - 1:
                    m = jnp.max(tops[u], axis=0, keepdims=True)
                    maxima[u] = jnp.broadcast_to(m, (8, mb))

            def weigh(u, c):
                step, h = t + u // hpg, u % hpg
                m = maxima[u]
                if sum_log:
                    m = jnp.minimum(m, m + sum_log[-1])
                if len(top_log) >= PACE:
                    m = jnp.minimum(m, jnp.maximum(m, top_log[-PACE]))
                keys = slice(c * CK, (c + 1) * CK)
                p = jnp.exp2(sc_v[u % 2][keys, :] - jnp.tile(m, (CK // 8, 1)))
                total = _fold_rows(jnp.add, p)
                sums[u] = sums[u] + total if c else total
                sum_log.append(sums[u])
                vt = vt_v[step // SPLIT, h * dh // 2 : (h + 1) * dh // 2, keys]
                o = _dot(_unpack(vt), p.astype(BF16))
                accs[u] = accs[u] + o if c else o
                if c == n_ck - 1:
                    total = jnp.sum(sums[u], axis=0, keepdims=True)
                    outs.append(accs[u] * (1.0 / total))
                    if h == hpg - 1:
                        o_v[step, 0:mb, :] = jnp.concatenate(outs[-hpg:], axis=0).T

            for i in range(lo, hi):
                ahead = i + n_ck + LAG
                if ahead < n_units * n_ck:
                    score(*divmod(ahead, n_ck))
                if i >= 0:
                    weigh(*divmod(i, n_ck))
            if hi < n_units * n_ck:
                u = hi // n_ck
                carry_v[0:8], carry_v[8:16] = maxima[u], tops[u + 1]
                carry_v[16:24], carry_v[24 : 24 + dh] = sums[u], accs[u]

        with _scope("att0"):
            attend(0, -n_ck - LAG, CUT, hpg)

        @pl.loop(0, n_step - 1)
        def _(t):
            with _scope("att"):
                attend(t, CUT, CUT + hpg * n_ck, 2 * hpg)

        def o_block(r, c):
            return jnp.concatenate(
                [o_v[(c * gpb + g) * SPLIT + r, 0:mb, :] for g in range(gpb)], axis=1
            )

        def emit_s(r, c, v):
            a_v[r * SPLIT + c, 0:mb, :] = v

        with _scope("o"):
            for c in range(SPLIT):
                wo_copy(c).wait()
            attend(n_step - 1, CUT, hpg * n_ck, hpg)
            _strassen(
                lambda i: _dot(_operand(_A_TERMS, i, o_block), square_weight(i)),
                emit_s,
                temporaries(),
            )

    pl.run_scoped(
        attention_branch,
        pltpu.VMEM((n_grp * SPLIT, LANES // 2, mb), U32),
        pltpu.VMEM((n_grp, S // 2, LANES), U32),
        pltpu.VMEM((n_grp, LANES // 2, S), U32),
        [pltpu.VMEM((S, mb), F32)] * 2,
        pltpu.VMEM((24 + dh, mb), F32),
        pltpu.VMEM((n_grp * SPLIT, mb + 8, LANES), F32),
    )

    def ffn_branch(h_v, wc_v):
        sb = mb // SPLIT
        for copy in ffn_copies():
            copy.wait()

        @pl.loop(0, n_fc)
        def _(j):
            def wd_operands(i):
                tile, phase = divmod(i, 3)
                if phase != 1 or tile >= (LANES // 16) * gpb:
                    return
                row, col = tile // gpb * 16, tile % gpb * LANES
                operands = _all_operands(
                    _B_TERMS,
                    lambda r, c: wd_v[
                        j, pl.ds(r * LANES + row, 16), pl.ds(c * kb + col, LANES)
                    ],
                )
                for n, w in enumerate(operands):
                    wc_v[n, j, pl.ds(row // 2, 8), pl.ds(col, LANES)] = _pack(w)

            def emit(r, c, v):
                h = _sigmoid(v[:, :LANES]) * v[:, LANES:]
                for q in range(SPLIT):
                    h_v[(r * SPLIT + q) * SPLIT + c, j, 0:sb, :] = h[q * sb : (q + 1) * sb]

            with _scope("gu"):
                paired_projection(j, emit, wd_operands)

        def out_copy(i):
            rows = pl.ds(pl.multiple_of(i * mb, mb), mb)
            return pltpu.make_async_copy(x_v.at[rows], out_hbm.at[rows], out_sem.at[i])

        @pl.loop(0, SPLIT)
        def _(b):
            def h_block(r, c):
                n = (b * SPLIT + r) * SPLIT + c
                return jnp.concatenate([h_v[n, j, 0:sb, :] for j in range(n_fc)], axis=1)

            def product(i):
                w = jnp.concatenate([wc_v[i, j] for j in range(n_fc)], axis=0)
                return _dot(_operand(_A_TERMS, i, h_block), _unpack(w))

            def emit(r, c, d):
                rows = pl.ds(pl.multiple_of(b * mb + r * sb, sb), sb)
                cols = pl.ds(c * kb, kb)
                s = a_v[b * SPLIT + c, r * sb : (r + 1) * sb, :]
                y = x_v[rows, cols].astype(F32) + s * (d * _sigmoid(d))
                x_v[rows, cols] = y.astype(x_v.dtype)

            with _scope("down"):
                _strassen(product, emit)
            out_copy(b).start()

        with _scope("fin"):
            for i in range(SPLIT):
                out_copy(i).wait()

    pl.run_scoped(
        ffn_branch,
        pltpu.VMEM((SPLIT**3, n_fc, mb // SPLIT + H_PAD, LANES), F32),
        pltpu.VMEM((N_PROD, n_fc, LANES // 2, kb), U32),
    )


IN_FLIGHT = 3
LN_AT = (0, 2, 8, 11)
H_PAD = 8


@jax.jit
def pallas_recurrent_scan__softmax_full_mha__glu_gated_glu__prompt_kernel(
    A_x: jax.Array,
    A_wqkv: jax.Array,
    A_wo: jax.Array,
    B_x: jax.Array,
    B_w_gate: jax.Array,
    B_w_up: jax.Array,
    B_w_down: jax.Array,
):
    del B_x
    B, S, D = A_x.shape
    F = B_w_gate.shape[1]
    assert (B, S, D) == (1, 2048, 1024) and F % FC == 0
    mb, kb = S // SPLIT, D // SPLIT
    n_slots = 2 * max(F, D) // FC

    out = pl.pallas_call(
        _kernel,
        out_shape=jax.ShapeDtypeStruct((S, D), A_x.dtype),
        in_specs=[pl.BlockSpec(memory_space=pl.ANY)] * 6,
        out_specs=pl.BlockSpec(memory_space=pl.ANY),
        scratch_shapes=[
            pltpu.VMEM((S, D), A_x.dtype),
            pltpu.VMEM((n_slots, D, FC), BF16),
            pltpu.VMEM((SPLIT, D, kb), BF16),
            pltpu.VMEM((F // FC, FC, D), BF16),
            pltpu.VMEM((N_PROD, mb // 2, kb), U32),
            pltpu.VMEM((SPLIT * SPLIT, mb + 8, kb), F32),
            [pltpu.VMEM((1, mb, kb), F32)] * 25,
            pltpu.SMEM((1,), jnp.int32),
            pltpu.SemaphoreType.DMA((S // X_PIECE,)),
            pltpu.SemaphoreType.DMA((SPLIT,)),
            pltpu.SemaphoreType.DMA((n_slots,)),
            pltpu.SemaphoreType.DMA((SPLIT,)),
            pltpu.SemaphoreType.DMA((F // FC,)),
            pltpu.SemaphoreType.DMA((SPLIT,)),
        ],
        compiler_params=pltpu.CompilerParams(vmem_limit_bytes=124 * 2**20),
    )(A_x.reshape(S, D), A_wqkv, A_wo, B_w_gate, B_w_up, B_w_down)
    return out.reshape(B, S, D)
```

```python
import itertools
import math

import jax
import jax.numpy as jnp
from jax import lax
import jax.experimental.pallas as pl
import jax.experimental.pallas.tpu as pltpu

F32 = jnp.float32
BF16 = jnp.bfloat16
U32 = jnp.uint32

N_HEADS = 32
LN_EPS = 1e-5
LANES = 128
SPLIT = 4
N_PROD = 49
N_TMP = 25
FC = SPLIT * LANES
PAD = 8

BQ = 256
CK = 128
LAG = 4
CUT = 8
UNROLL = 4
VPU_CHUNKS = (10, 11)
EXP_PACE, KEY_PACE, SUM_PACE = 7, 5, 9

X_PIECE = 128
LN_BATCH = 32
LN_ROWS = 16

_START_UP = [
    line.split()
    for line in """
start x0 x1 x2 x3
wait x0
do 4
start q3
wait x1
do 4
wait x2
do 4
start x4
wait x3
do 4
start x5 k3
wait q3
do q0 q1 q7 q8
start x6 x7
wait k3 x4 x5
do 3 k0 5 k1
start q2
wait x6 x7
do 3 k7 5 k8
start k2 x8 x9 x10
wait q2
do q2 q3 q4 q5 q6 q9
start x11 x12 x13 x14 x15 q1 k1
wait k2 x8 x9 x10
do 1 k2 3 k3 2 k4 2 k5 2 k6 1 q10 q11 1 q12 q13 k9
start q0 k0
wait x11 x12 x13 x14 x15 q1 k1
do 1 k10 3 k11 3 k12 2 k13 2 q14 2 q15 3 k14 4 k15
start v0 v1 v2 v3
wait q0 k0
""".strip().split("\n")
]
_WAITS = [names for action, *names in _START_UP if action == "wait"]
_WAITS.append(["v0", "v1", "v2", "v3"])

_A_TERMS = (
    ((1, 0, 0), (1, 0, 1)),
    ((1, 0, 0),),
    ((1, 1, 0), (1, 1, 1)),
    ((1, 1, 1),),
    ((1, 0, 0), (1, 1, 1)),
    ((1, 1, 0), (-1, 0, 0)),
    ((1, 0, 1), (-1, 1, 1)),
)
_B_TERMS = (
    ((1, 1, 1),),
    ((1, 0, 1), (-1, 1, 1)),
    ((1, 0, 0),),
    ((1, 1, 0), (-1, 0, 0)),
    ((1, 0, 0), (1, 1, 1)),
    ((1, 0, 0), (1, 0, 1)),
    ((1, 1, 0), (1, 1, 1)),
)


def _signed_sum(terms, block):
    acc = None
    for sign, r, c in terms:
        b = block(r, c).astype(F32)
        acc = b if acc is None else (acc + b if sign > 0 else acc - b)
    return acc


def _operand(table, i, block):
    terms = [
        (s0 * s1, 2 * r0 + r1, 2 * c0 + c1)
        for (s0, r0, c0), (s1, r1, c1) in itertools.product(table[i // 7], table[i % 7])
    ]
    if len(terms) == 1:
        return block(*terms[0][1:]).astype(BF16)
    return _signed_sum(terms, block).astype(BF16)


def _all_operands(table, block):
    for outer in table:
        half = {
            (r, c): _signed_sum(outer, lambda i, j: block(2 * i + r, 2 * j + c))
            for r in range(2)
            for c in range(2)
        }
        for inner in table:
            yield _signed_sum(inner, lambda i, j: half[i, j]).astype(BF16)


def _combine(k, v, put, get):
    if k in (0, 2, 4):
        put(k, v)
        return None
    if k == 1:
        put(1, v)
        return 0, 1, get(0) + v
    if k == 3:
        put(3, v - get(0))
        return 1, 0, get(2) + v
    if k == 5:
        return 1, 1, get(1) - get(2) + get(4) + v
    return 0, 0, get(3) + get(4) + v


def _collector(emit, tmp=None):
    kept = {}

    def slots(base):
        def put(n, v):
            if tmp is None:
                kept[base + n] = v
            else:
                tmp[base + n][...] = v

        return put, lambda n: kept[base + n] if tmp is None else tmp[base + n][...]

    def take(i, product):
        inner = _combine(i % 7, product, *slots(0))
        if inner is not None:
            r, c, v = inner
            outer = _combine(i // 7, v, *slots(5 + 5 * (2 * r + c)))
            if outer is not None:
                emit(2 * outer[0] + r, 2 * outer[1] + c, outer[2])

    return take


def _strassen(product, emit, tmp=None):
    take = _collector(emit, tmp)
    for i in range(N_PROD):
        take(i, product(i))


def _advance(work, count=None):
    for _ in itertools.islice(work, count):
        pass


def _pack(x):
    return pltpu.bitcast(x, U32)


def _unpack(x):
    return pltpu.bitcast(x, BF16)


def _dot(a, b):
    return jnp.dot(a, b, preferred_element_type=F32)


def _sigmoid(x):
    return 0.5 * jnp.tanh(0.5 * x) + 0.5


def _after(x, y):
    return jnp.minimum(x, jnp.maximum(x, y))


def _fold_rows(op, x):
    r = x[0:8]
    for i in range(1, x.shape[0] // 8):
        r = op(r, x[8 * i : 8 * i + 8])
    return r


def _kernel(
    x_hbm, wqkv_hbm, wo_hbm, wg_hbm, wu_hbm, wd_hbm, out_hbm,
    x_v, w_v, wd_v, xc_v, a_v, tmp_v, zero_s,
    start_sem, ffn_sem, wo_sem, out_sem,
):
    S, D = x_v.shape
    n_fc = wd_v.shape[0]
    mb, kb = S // SPLIT, D // SPLIT
    dh = D // N_HEADS
    hpg = LANES // dh
    n_grp, gpb = D // LANES, kb // LANES
    n_qb, qpb = S // BQ, mb // BQ

    zero_s[0] = 0

    def temporaries(refs):
        zero = zero_s[0]
        return [t.at[zero] for t in refs]

    def square_copy(src, mat, c, dst, sem):
        cols = pl.ds(mat * D + c * kb, kb)
        return pltpu.make_async_copy(src.at[:, cols], dst.at[c], sem)

    def square_weight(ref, i):
        return _operand(_B_TERMS, i, lambda r, c: ref[c, r * kb : (r + 1) * kb, :])

    def ffn_copies():
        for j in range(n_fc):
            part = pl.ds(j * FC, FC)
            yield pltpu.make_async_copy(wg_hbm.at[:, part], w_v.at[2 * j], ffn_sem)
            yield pltpu.make_async_copy(wu_hbm.at[:, part], w_v.at[2 * j + 1], ffn_sem)
            yield pltpu.make_async_copy(wd_hbm.at[part], wd_v.at[j], ffn_sem)

    def attention_branch(
        wqkv_v, wo_v, tmp2_v, early_v, ln_v, qt_v, k_v, vt_v, sc_v, carry_v, o_v
    ):
        def normalise(base, after):
            zero = zero_s[0]
            centred = ln_v[base // LN_BATCH % len(ln_v)]
            rows = range(base, base + LN_BATCH, LN_ROWS)
            mean = [
                jnp.mean(x_v[i : i + LN_ROWS, :].astype(F32), axis=-1, keepdims=True)
                for i in rows
            ]
            if after is not None:
                mean = [_after(m, next(after)) for m in mean]
            scale = []
            for i, m in zip(rows, mean):
                again = pl.ds(pl.multiple_of(i + zero, LN_ROWS), LN_ROWS)
                x = x_v[again, :].astype(F32) - m
                var = jnp.mean(x * x, axis=-1, keepdims=True)
                scale.append(lax.rsqrt(var + LN_EPS))
                centred[zero, i - base : i - base + LN_ROWS, :] = x
            for i, g in zip(rows, scale):
                xn = centred[zero, i - base : i - base + LN_ROWS, :] * g
                r, row = divmod(i, mb)
                for c in range(SPLIT):
                    a_v[r * SPLIT + c, row : row + LN_ROWS, :] = xn[
                        :, c * kb : (c + 1) * kb
                    ]

        def copy(name):
            sem = start_sem.at[[name in names for names in _WAITS].index(True)]
            n = int(name[1:])
            if name[0] == "x":
                rows = pl.ds(n * X_PIECE, X_PIECE)
                return pltpu.make_async_copy(x_hbm.at[rows], x_v.at[rows], sem)
            mat = "qkv".index(name[0])
            return square_copy(wqkv_hbm, mat, n, wqkv_v[mat], sem)

        def emit_q(r, c, v):
            t = _pack((v * (dh**-0.5 * math.log2(math.e))).astype(BF16).T)
            for g in range(gpb):
                for b in range(qpb):
                    qt_v[(c * gpb + g) * n_qb + r * qpb + b] = t[
                        g * LANES // 2 : (g + 1) * LANES // 2, b * BQ : (b + 1) * BQ
                    ]

        def emit_k(r, c, v):
            t = _pack(v.astype(BF16))
            for g in range(gpb):
                k_v[c * gpb + g, r * mb // 2 : (r + 1) * mb // 2, :] = t[
                    :, g * LANES : (g + 1) * LANES
                ]

        def emit_v(r, c, v):
            t = _pack(v.astype(BF16).T)
            for g in range(gpb):
                vt_v[c * gpb + g, :, r * mb : (r + 1) * mb] = t[
                    g * LANES // 2 : (g + 1) * LANES // 2
                ]

        take = (
            _collector(emit_q, temporaries(tmp_v)),
            _collector(emit_k, temporaries(tmp2_v)),
        )
        taken, early = [0, 0], [{}, {}]

        def qk_product(mat, i, offset=0):
            if mat == 0:
                a = _operand(_A_TERMS, i, lambda r, c: a_v[r * SPLIT + c, 0:mb, :])
                xc_v[i] = _pack(a)
            else:
                a = _unpack(xc_v[i + offset])
            result = _dot(a, square_weight(wqkv_v[mat], i))
            if i > taken[mat]:
                early[mat][i] = early_v.at[zero_s[0] + len(early[0]) + len(early[1])]
                early[mat][i][...] = result
                return result
            take[mat](i, result)
            taken[mat] += 1
            while taken[mat] in early[mat]:
                take[mat](taken[mat], early[mat][taken[mat]][...])
                taken[mat] += 1
            return result

        ln_batches = iter(range(0, S, LN_BATCH))
        for action, *names in _START_UP:
            beside = None
            for name in names:
                if action == "start":
                    copy(name).start()
                elif action == "wait":
                    copy(name).wait()
                elif name.isdigit():
                    n = int(name) * LN_BATCH // LN_ROWS
                    after = None
                    if beside is not None:
                        after = (beside[i * mb // n :][:LN_ROWS, :1] for i in range(n))
                    for base in itertools.islice(ln_batches, int(name)):
                        normalise(base, after)
                else:
                    beside = qk_product("qk".index(name[0]), int(name[1:]))
        assert next(ln_batches, None) is None
        for i in range(taken[0], N_PROD):
            qk_product(0, i)
        for i in range(taken[1], N_PROD):
            qk_product(1, i, zero_s[0])

        for name in _WAITS[-1]:
            copy(name).wait()
        _strassen(
            lambda i: _dot(_unpack(xc_v[i]), square_weight(wqkv_v[2], i)),
            emit_v,
            temporaries(tmp_v),
        )

        for c in range(SPLIT):
            square_copy(wo_hbm, 0, c, wo_v, wo_sem).start()
        for ffn_copy in ffn_copies():
            ffn_copy.start()

        n_ck = S // CK
        n_step = n_grp * n_qb

        def attend(t, lo, hi, n_units):
            queries, maxima, tops, sums, accs = {}, {}, {}, {}, {}
            top_log, partial, outs = [], [], []
            if lo > 0:
                maxima[0], tops[1] = carry_v[0:8], carry_v[8:16]
                sums[0], accs[0] = carry_v[16:24], carry_v[24 : 24 + dh]

            def score_on_vpu(u, c):
                step, h = t + u // hpg, u % hpg
                j, d0 = divmod(8 * c, dh)
                q = _unpack(qt_v[step, pl.ds((h * dh + d0) // 16 * 8, 8), :]).astype(F32)
                q = q[d0 % 16 : d0 % 16 + 8]
                if len(partial) >= SUM_PACE:
                    q = _after(q, partial[-SUM_PACE])
                row = (VPU_CHUNKS[j // 2] + 1) * CK - 16
                k = _unpack(k_v[step // n_qb, pl.ds(row // 2, 8), :]).astype(F32)
                k, row = k[j % 2 * 8 : j % 2 * 8 + 8], row + j % 2 * 8
                if len(top_log) >= KEY_PACE:
                    k = _after(k, top_log[-KEY_PACE][:, :LANES])
                for d in range(8):
                    lane = h * dh + d0 + d
                    term = k[:, lane : lane + 1] * q[d : d + 1]
                    partial.append(partial[-1] + term if d0 + d else term)
                if d0 + 8 == dh:
                    sc_v[u % 2][row : row + 8, :] = partial[-1]
                    tops[u] = jnp.maximum(tops[u], partial[-1])

            def score(u, c):
                step, h = t + u // hpg, u % hpg
                if u not in queries:
                    r0, r1 = h * dh // 2, (h + 1) * dh // 2
                    parts = [qt_v[step, r0:r1, :]]
                    if r0:
                        parts.insert(0, jnp.zeros((r0, BQ), U32))
                    if r1 < LANES // 2:
                        parts.append(jnp.zeros((LANES // 2 - r1, BQ), U32))
                    queries[u] = _unpack(jnp.concatenate(parts, axis=0))
                n = CK - 16 * (c in VPU_CHUNKS)
                k = k_v[step // n_qb, pl.ds(c * CK // 2, n // 2), :]
                s = _dot(_unpack(k), queries[u])
                sc_v[u % 2][pl.ds(c * CK, n), :] = s
                top = _fold_rows(jnp.maximum, s)
                tops[u] = jnp.maximum(tops[u], top) if c else top
                top_log.append(tops[u])
                score_on_vpu(u, c)
                if c == n_ck - 1:
                    m = jnp.max(tops[u], axis=0, keepdims=True)
                    maxima[u] = jnp.broadcast_to(m, (8, BQ))

            def weigh(u, c):
                step, h = t + u // hpg, u % hpg
                m = maxima[u]
                if len(top_log) >= EXP_PACE:
                    m = _after(m, top_log[-EXP_PACE])
                keys = slice(c * CK, (c + 1) * CK)
                p = jnp.exp2(sc_v[u % 2][keys, :] - jnp.tile(m, (CK // 8, 1)))
                total = _fold_rows(jnp.add, p)
                sums[u] = sums[u] + total if c else total
                vt = vt_v[step // n_qb, h * dh // 2 : (h + 1) * dh // 2, keys]
                o = _dot(_unpack(vt), p.astype(BF16))
                accs[u] = accs[u] + o if c else o
                if c == n_ck - 1:
                    total = jnp.sum(sums[u], axis=0, keepdims=True)
                    outs.append(accs[u] * (1.0 / total))
                    if h == hpg - 1:
                        o_v[step, 0:BQ, :] = jnp.concatenate(outs[-hpg:], axis=0).T

            for i in range(lo, hi):
                ahead = i + n_ck + LAG
                if ahead < n_units * n_ck:
                    score(*divmod(ahead, n_ck))
                if i >= 0:
                    weigh(*divmod(i, n_ck))
                yield
            if hi < n_units * n_ck:
                u = hi // n_ck
                carry_v[0:8], carry_v[8:16] = maxima[u], tops[u + 1]
                carry_v[16:24], carry_v[24 : 24 + dh] = sums[u], accs[u]

        _advance(attend(0, -n_ck - LAG, CUT, hpg))

        @pl.loop(0, n_step - UNROLL, step=UNROLL)
        def _(t):
            _advance(attend(t, CUT, CUT + UNROLL * hpg * n_ck, (UNROLL + 1) * hpg))

        for c in range(SPLIT):
            square_copy(wo_hbm, 0, c, wo_v, wo_sem).wait()
        end = UNROLL * hpg * n_ck
        rest = attend(n_step - UNROLL, CUT, end, UNROLL * hpg)
        _advance(rest, end - CUT - n_ck - LAG)

        def o_block(r, c):
            return jnp.block(
                [
                    [o_v[(c * gpb + g) * n_qb + r * qpb + b, 0:BQ, :] for g in range(gpb)]
                    for b in range(qpb)
                ]
            )

        def o_product(i):
            _advance(rest, 2 if i < 14 else None)
            return _dot(_operand(_A_TERMS, i, o_block), square_weight(wo_v, i))

        def emit_s(r, c, v):
            a_v[r * SPLIT + c, 0:mb, :] = v

        _strassen(o_product, emit_s, temporaries(tmp_v))

    pl.run_scoped(
        attention_branch,
        [pltpu.VMEM((SPLIT, D, kb), BF16)] * 3,
        pltpu.VMEM((SPLIT, D, kb), BF16),
        [pltpu.VMEM((1, mb, kb), F32)] * N_TMP,
        pltpu.VMEM((4, mb, kb), F32),
        [pltpu.VMEM((1, LN_BATCH, D), F32)] * 16,
        pltpu.VMEM((n_grp * n_qb, LANES // 2, BQ), U32),
        pltpu.VMEM((n_grp, S // 2, LANES), U32),
        pltpu.VMEM((n_grp, LANES // 2, S), U32),
        [pltpu.VMEM((S, BQ), F32)] * 2,
        pltpu.VMEM((24 + dh, BQ), F32),
        pltpu.VMEM((n_grp * n_qb, BQ + PAD, LANES), F32),
    )

    def ffn_branch(h_v, wc_v):
        sb = mb // SPLIT
        for ffn_copy in ffn_copies():
            ffn_copy.wait()

        @pl.loop(0, n_fc)
        def _(j):
            def wd_operands():
                for row in range(0, LANES, 16):
                    for col in range(0, kb, LANES):
                        operands = _all_operands(
                            _B_TERMS,
                            lambda r, c: wd_v[
                                j, pl.ds(r * LANES + row, 16), pl.ds(c * kb + col, LANES)
                            ],
                        )
                        for n, w in enumerate(operands):
                            wc_v[n, j, pl.ds(row // 2, 8), pl.ds(col, LANES)] = _pack(w)
                            yield

            side_work = wd_operands()

            def w_block(r, c):
                rows, cols = pl.ds(r * kb, kb), pl.ds(c * LANES, LANES)
                return jnp.concatenate([w_v[2 * j + i, rows, cols] for i in range(2)], 1)

            def product(i):
                result = _dot(_unpack(xc_v[i]), _operand(_B_TERMS, i, w_block))
                if i + 1 < N_PROD:
                    terms = len(_B_TERMS[(i + 1) // 7]) * len(_B_TERMS[(i + 1) % 7])
                    _advance(side_work, (31, 22, 10)[terms // 2])
                return result

            def emit(r, c, v):
                h = _sigmoid(v[:, :LANES]) * v[:, LANES:]
                for q in range(SPLIT):
                    h_v[(r * SPLIT + q) * SPLIT + c, j, 0:sb, :] = h[q * sb : (q + 1) * sb]

            _strassen(product, emit, temporaries(tmp_v))
            _advance(side_work)

        def out_copy(b, r, c):
            rows = pl.ds(pl.multiple_of(b * mb + r * mb // 2, mb // 2), mb // 2)
            cols = pl.ds(c * D // 2, D // 2)
            return pltpu.make_async_copy(
                x_v.at[rows, cols], out_hbm.at[rows, cols], out_sem
            )

        @pl.loop(0, SPLIT)
        def _(b):
            def h_block(r, c):
                n = (b * SPLIT + r) * SPLIT + c
                return jnp.concatenate([h_v[n, j, 0:sb, :] for j in range(n_fc)], axis=1)

            def product(i):
                if i == 43:
                    for r, c in ((0, 1), (1, 0), (1, 1)):
                        out_copy(b, r, c).start()
                w = jnp.concatenate([wc_v[i, j] for j in range(n_fc)], axis=0)
                return _dot(_operand(_A_TERMS, i, h_block), _unpack(w))

            def emit(r, c, d):
                rows = pl.ds(pl.multiple_of(b * mb + r * sb, sb), sb)
                cols = pl.ds(c * kb, kb)
                s = a_v[b * SPLIT + c, r * sb : (r + 1) * sb, :]
                y = x_v[rows, cols].astype(F32) + s * (d * _sigmoid(d))
                x_v[rows, cols] = y.astype(x_v.dtype)

            _strassen(product, emit)
            out_copy(b, 0, 0).start()

        for b, r, c in itertools.product(range(SPLIT), range(2), range(2)):
            out_copy(b, r, c).wait()

    pl.run_scoped(
        ffn_branch,
        pltpu.VMEM((SPLIT**3, n_fc, mb // SPLIT + PAD, LANES), F32),
        pltpu.VMEM((N_PROD, n_fc, LANES // 2, kb), U32),
    )


@jax.jit
def pallas_recurrent_scan__softmax_full_mha__glu_gated_glu__prompt_kernel(
    A_x: jax.Array,
    A_wqkv: jax.Array,
    A_wo: jax.Array,
    B_x: jax.Array,
    B_w_gate: jax.Array,
    B_w_up: jax.Array,
    B_w_down: jax.Array,
):
    del B_x
    B, S, D = A_x.shape
    F = B_w_gate.shape[1]
    assert (B, S, D) == (1, 2048, 1024) and F % FC == 0
    mb, kb = S // SPLIT, D // SPLIT

    out = pl.pallas_call(
        _kernel,
        out_shape=jax.ShapeDtypeStruct((S, D), A_x.dtype),
        in_specs=[pl.BlockSpec(memory_space=pl.ANY)] * 6,
        out_specs=pl.BlockSpec(memory_space=pl.ANY),
        scratch_shapes=[
            pltpu.VMEM((S, D), A_x.dtype),
            pltpu.VMEM((2 * F // FC, D, FC), BF16),
            pltpu.VMEM((F // FC, FC, D), BF16),
            pltpu.VMEM((N_PROD, mb // 2, kb), U32),
            pltpu.VMEM((SPLIT * SPLIT, mb + PAD, kb), F32),
            [pltpu.VMEM((1, mb, kb), F32)] * N_TMP,
            pltpu.SMEM((1,), jnp.int32),
            pltpu.SemaphoreType.DMA((len(_WAITS),)),
            pltpu.SemaphoreType.DMA(()),
            pltpu.SemaphoreType.DMA(()),
            pltpu.SemaphoreType.DMA(()),
        ],
        compiler_params=pltpu.CompilerParams(vmem_limit_bytes=124 * 2**20),
    )(A_x.reshape(S, D), A_wqkv, A_wo, B_w_gate, B_w_up, B_w_down)
    return out.reshape(B, S, D)
```

```python
import functools
import itertools
import math

import jax
import jax.numpy as jnp
from jax import lax
import jax.experimental.pallas as pl
import jax.experimental.pallas.tpu as pltpu

F32 = jnp.float32
BF16 = jnp.bfloat16
U32 = jnp.uint32

N_HEADS = 32
LN_EPS = 1e-5
LANES = 128
ROWS = 256
FC = 4 * LANES
PAD = 8

CK = 128
LAG = 4
CUT = 8
UNROLL = 4
VPU_CHUNKS = (10, 11)
EXP_PACE, KEY_PACE, SUM_PACE = 7, 5, 9

X_PIECE = 128
LN_BATCH = 32
LN_ROWS = 16

_START_UP = [
    line.split()
    for line in """
start x0 x1
wait x0
do nnnn
start w145
wait x1
do nnnn ff
start x2 x3
wait w145
do fff pp
start w156
wait x2 x3
do nnnnnnnn ff
start x4 x5
wait w156
do fff ppp
start w167
wait x4 x5
do nnn pnnnnn pff
start x6 x7
wait w167
do fff ppp
start w178 w046
wait x6 x7
do nn pnn pnn pnn f p f
start w068 x8 x9 x10 x11
wait w178 w046
do fff pf pf pf pff pf pf pf pf pf ppp
start x12 x13 x14 x15 w004
wait w068 x8 x9 x10 x11
do f pf pf pf pfn pnn pn pn pffn pffn pfn pn pn p
start w104
wait x12 x13 x14 x15 w004
do f pf pf pffnn pnn pnn pff pf pf pf pnn pn pn p pnn pnn pffn pffn pfnn pnn pnn p
wait w104
block f pff pff pf pf pff pf pf pff pff pff pff pf pf pf pff pf pp {forms}
block ppppppp {forms} ppppppp pff pf pff pff pf p p pff pff
block pf p p pff p p pff pff p pf ppppppp pppppppppppppppppppppppppp a
""".format(forms="pff pf pff pff pf p p pff pff pf p p pff p p pff pff p pf")
    .strip()
    .split("\n")
]
_WAITS = [names for action, *names in _START_UP if action == "wait"]
_TWELVE_PIECES = "11101110011001000110001000"
_LAST_UNIT = "10101011010110110101101100"
_DOWN_PIECES = "44444443344334343443333321"

_A_TERMS = (
    ((1, 0, 0), (1, 0, 1)),
    ((1, 0, 0),),
    ((1, 1, 0), (1, 1, 1)),
    ((1, 1, 1),),
    ((1, 0, 0), (1, 1, 1)),
    ((1, 1, 0), (-1, 0, 0)),
    ((1, 0, 1), (-1, 1, 1)),
)
_B_TERMS = (
    ((1, 1, 1),),
    ((1, 0, 1), (-1, 1, 1)),
    ((1, 0, 0),),
    ((1, 1, 0), (-1, 0, 0)),
    ((1, 0, 0), (1, 1, 1)),
    ((1, 0, 0), (1, 0, 1)),
    ((1, 1, 0), (1, 1, 1)),
)


def _strassen_combine(k, v, slots):
    if k in (0, 1, 2, 4):
        slots[k][...] = v
    if k == 1:
        return 0, 1, slots[0][...] + v
    if k == 3:
        slots[3][...] = v - slots[0][...]
        return 1, 0, slots[2][...] + v
    if k == 5:
        return 1, 1, slots[1][...] - slots[2][...] + slots[4][...] + v
    if k == 6:
        return 0, 0, slots[3][...] + slots[4][...] + v
    return None


def _signed_sum(terms, block):
    assert terms[0][0] == 1
    acc = None
    for sign, *key in terms:
        b = block(*key).astype(F32)
        acc = b if acc is None else (acc + b if sign > 0 else acc - b)
    return acc


def _after(x, y):
    return jnp.minimum(x, jnp.maximum(x, y)) if len(y) else x


def _left_forms(o, block, after):
    a0, a1 = (_signed_sum(_A_TERMS[o], functools.partial(block, k)) for k in range(2))
    a0 = _after(a0, after)
    h = -0.5 * a0
    return a0, a1 + h, a1 - h


def _right_forms(o, block, after):
    b0, b1 = (_signed_sum(_B_TERMS[o], functools.partial(block, k)) for k in range(2))
    b1 = _after(b1, after)
    h = 0.5 * b1
    return b1, h + b0, h - b0


def _hopcroft_kerr(order):
    t_of = (0, 1, 2, 0, 2)

    def left(sign, i, k):
        sign = sign if k < 2 else -sign
        return [(sign, i, k)] if i < 4 else [(sign, 0, k), (-sign, 1, k)]

    def right(sign, j, k):
        sign = sign if k else -sign
        return [(sign, j, k)] if j < 4 else [(sign, 0, k), (sign, 1, k)]

    def diagonal(i):
        l, m = (t_of[i] + 1) % 3, (t_of[i] + 2) % 3
        u = left(1, i, l), right(1, i, m), f"u{i}"
        v = left(1, i, m), right(1, i, l), f"v{i}"
        yield *(u if l else v), None
        yield *(v if l else u), (i, i, [(1, f"u{i}"), (-1, f"v{i}")], None)

    def pair(i, j, names=("p", "q"), row=None, more=((), ())):
        k, l, m, r = t_of[i], t_of[j], f"m{i}{j}", i if row is None else row
        assert l == (k + 1) % 3
        upper = [(1, f"v{i}"), (-1, f"v{j}"), *more[0], (1, m), (1, names[0])]
        lower = [(1, f"u{i}"), (-1, f"u{j}"), *more[1], (1, m), (1, names[1])]
        yield left(1, i, l) + left(1, j, k), right(1, i, l) + right(-1, j, k), m, None
        yield (
            left(1, i, k) + left(-1, j, k), right(1, i, l) + right(1, j, l),
            names[0], (r, j, upper, f"c{r}{j}"),
        )
        yield (
            left(1, i, l) + left(-1, j, l), right(1, i, k) + right(1, j, k),
            names[1], (j, r, lower, f"c{j}{r}"),
        )

    groups = {str(i): diagonal(i) for i in range(4)}
    groups.update({f"{i}{j}": pair(i, j) for i, j in ((1, 2), (2, 0), (3, 1), (2, 3))})
    groups["01"] = pair(0, 1, names=("u4", "v4"))
    groups["43"] = pair(4, 3, row=0, more=([(1, "c13")], [(-1, "c31")]))

    def plus_first(terms):
        n = [sign for sign, *_ in terms].index(1)
        return [terms[n]] + terms[:n] + terms[n + 1 :]

    steps, signs = [], {}
    for a, b, name, result in (next(groups[g]) for g in order.split()):
        flips = [max(sign for sign, *_ in terms) for terms in (a, b)]
        a, b = (
            plus_first([(sign * flip, *key) for sign, *key in terms])
            for terms, flip in zip((a, b), flips)
        )
        signs[name] = flips[0] * flips[1]
        if result is not None:
            i, j, terms, c = result
            result = i, j, plus_first([(s * signs.get(n, 1), n) for s, n in terms]), c
        steps.append((a, b, name, result))
    return steps


_HK = _hopcroft_kerr(
    "1 2 0 1 0 01 2 01 01 12 20 12 12 3 20 3 20 31 23 31 31 23 43 23 43 43"
)
_HK_ROW_BY_ROW = _hopcroft_kerr(
    "0 0 1 01 1 01 01 2 12 2 12 12 20 20 20 3 31 3 23 31 31 23 43 23 43 43"
)
_HK_KEPT = sorted(
    {n for *_, name, result in _HK if result for _, n in result[2] if n != name}
)
N_PROD = 7 * len(_HK)


def _block_product(product, emit, kept, products=range(N_PROD), steps=_HK, amend=None):
    inner, outer = dict(zip(_HK_KEPT, kept[0])), kept[1]
    for number in products:
        o, s = divmod(number, len(steps))
        *_, name, result = steps[s]
        v = product(o, s)
        if name in inner:
            inner[name][...] = v
        if result is None:
            continue
        i, j, terms, c = result
        v = _signed_sum(terms, lambda n: v if n == name else inner[n][...])
        if c in inner:
            inner[c][...] = v
        if amend is not None:
            v = amend(o, i, j, v)
        done = _strassen_combine(o, v, outer[4 * i + j])
        if done is not None:
            emit(4 * done[0] + i, 4 * done[1] + j, done[2])


def _kept_shapes(width, slots=5):
    block = pltpu.VMEM((1, ROWS, width), F32)
    return [block] * len(_HK_KEPT), [[block] * slots] * 16


def _advance(work, count=None):
    for _ in itertools.islice(work, count):
        pass


def _paced(work):
    next(work)
    left = [True]

    def step(y):
        if left and y is not None:
            try:
                work.send(y)
            except StopIteration:
                left.clear()
        return not left

    return step


def _pack(x):
    return pltpu.bitcast(x, U32)


def _unpack(x):
    return pltpu.bitcast(x, BF16)


def _dot(a, b):
    return jnp.dot(a, b, preferred_element_type=F32)


def _fold_rows(op, x):
    r = x[0:8]
    for i in range(1, x.shape[0] // 8):
        r = op(r, x[8 * i : 8 * i + 8])
    return r


def _kernel(
    x_hbm, wqkv_hbm, wo_hbm, wg_hbm, wu_hbm, wd_hbm, out_hbm,
    x_v, w_v, wd_v, xf_v, a_v, zero_s,
    start_sem, w_sem, late_sem, out_sem,
):
    S, D = x_v.shape
    n_fc = wd_v.shape[0] // FC
    kb = D // 4
    dh = D // N_HEADS
    hpg = LANES // dh
    n_grp, gpb = D // LANES, kb // LANES
    n_qb = S // ROWS

    zero_s[0] = 0

    def temporaries(refs):
        zero = zero_s[0]
        return [t.at[zero] for t in refs[0]], [[t.at[zero] for t in r] for r in refs[1]]

    def own_block(n):
        return pl.when(zero_s[0] <= n)

    def gate_up_copies(j):
        cols = pl.ds(pl.multiple_of(j * FC, FC), FC)
        for n, src in enumerate((wg_hbm, wu_hbm)):
            yield pltpu.make_async_copy(src.at[:, cols], w_v.at[j % 2, n], w_sem.at[j % 2])

    def operands(form_v, left_block, weights):
        zero = zero_s[0]
        n_part = gpb + weights.shape[1] // D
        ready, in_use = [], [0]

        def make_forms():
            for o, i, part in itertools.product(range(7), range(4), range(n_part)):
                after = yield
                assert in_use[0] >= o - 1

                def a_block(k, r, c):
                    return left_block(4 * r + i, (2 * c + k) * gpb + part)

                def w_block(k, r, c):
                    col = (part - gpb) * D + (4 * c + i) * LANES
                    return weights[pl.ds((2 * r + k) * kb, kb), pl.ds(col, LANES)]

                if part < gpb:
                    forms = _left_forms(o, a_block, after)
                else:
                    forms = _right_forms(o, w_block, after)
                for k, f in enumerate(forms):
                    form_v[o % 2][zero, 3 * i + k, part, 0:ROWS, :] = f
                ready.append((o, i, part))

        def multiply(o, left, right, mats):
            in_use[0] = o

            def form(part, i, k):
                assert (o, i, part) in ready
                return form_v[o % 2][zero, 3 * i + k, part, 0:ROWS, :]

            a, w = (
                [_signed_sum(terms, functools.partial(form, part)) for part in parts]
                for terms, parts in ((left, range(gpb)), (right, [gpb + m for m in mats]))
            )
            a_bf16, w = (jnp.concatenate(x, axis=1).astype(BF16) for x in (a, w))
            return a, _dot(a_bf16, w)

        return _paced(make_forms()), multiply

    n_ck = S // CK
    n_step = n_grp * n_qb

    def attend(refs, o_v, t, lo, hi, n_units):
        qt_v, k_v, vt_v, sc_v, carry_v = refs
        queries, maxima, tops, sums, accs = {}, {}, {}, {}, {}
        top_log, partial, outs = [], [], []
        if lo > 0:
            maxima[0], tops[1] = carry_v[0:8], carry_v[8:16]
            sums[0], accs[0] = carry_v[16:24], carry_v[24 : 24 + dh]

        def score_on_vpu(u, c):
            step, h = t + u // hpg, u % hpg
            j, d0 = divmod(8 * c, dh)
            q = _unpack(qt_v[step, pl.ds((h * dh + d0) // 16 * 8, 8), :]).astype(F32)
            q = q[d0 % 16 : d0 % 16 + 8]
            if len(partial) >= SUM_PACE:
                q = _after(q, partial[-SUM_PACE])
            row = (VPU_CHUNKS[j // 2] + 1) * CK - 16
            k = _unpack(k_v[step // n_qb, pl.ds(row // 2, 8), :]).astype(F32)
            k, row = k[j % 2 * 8 : j % 2 * 8 + 8], row + j % 2 * 8
            if len(top_log) >= KEY_PACE:
                k = _after(k, top_log[-KEY_PACE][:, :LANES])
            for d in range(8):
                lane = h * dh + d0 + d
                term = k[:, lane : lane + 1] * q[d : d + 1]
                partial.append(partial[-1] + term if d0 + d else term)
            if d0 + 8 == dh:
                sc_v[u % 2][row : row + 8, :] = partial[-1]
                tops[u] = jnp.maximum(tops[u], partial[-1])

        def score(u, c):
            step, h = t + u // hpg, u % hpg
            if u not in queries:
                r0, r1 = h * dh // 2, (h + 1) * dh // 2
                parts = [qt_v[step, r0:r1, :]]
                if r0:
                    parts.insert(0, jnp.zeros((r0, ROWS), U32))
                if r1 < LANES // 2:
                    parts.append(jnp.zeros((LANES // 2 - r1, ROWS), U32))
                queries[u] = _unpack(jnp.concatenate(parts, axis=0))
            n = CK - 16 * (c in VPU_CHUNKS)
            k = k_v[step // n_qb, pl.ds(c * CK // 2, n // 2), :]
            s = _dot(_unpack(k), queries[u])
            sc_v[u % 2][pl.ds(c * CK, n), :] = s
            top = _fold_rows(jnp.maximum, s)
            tops[u] = jnp.maximum(tops[u], top) if c else top
            top_log.append(tops[u])
            score_on_vpu(u, c)
            if c == n_ck - 1:
                m = jnp.max(tops[u], axis=0, keepdims=True)
                maxima[u] = jnp.broadcast_to(m, (8, ROWS))

        def weigh(u, c):
            step, h = t + u // hpg, u % hpg
            m = maxima[u]
            if len(top_log) >= EXP_PACE:
                m = _after(m, top_log[-EXP_PACE])
            keys = slice(c * CK, (c + 1) * CK)
            p = jnp.exp2(sc_v[u % 2][keys, :] - jnp.tile(m, (CK // 8, 1)))
            total = _fold_rows(jnp.add, p)
            sums[u] = sums[u] + total if c else total
            vt = vt_v[step // n_qb, h * dh // 2 : (h + 1) * dh // 2, keys]
            o = _dot(_unpack(vt), p.astype(BF16))
            accs[u] = accs[u] + o if c else o
            if c == n_ck - 1:
                total = jnp.sum(sums[u], axis=0, keepdims=True)
                outs.append(accs[u] * (1.0 / total))
                if h == hpg - 1:
                    o_v[step, 0:ROWS, :] = jnp.concatenate(outs[-hpg:], axis=0).T

        for i in range(lo, hi):
            ahead = i + n_ck + LAG
            if ahead < n_units * n_ck:
                score(*divmod(ahead, n_ck))
            if i >= 0:
                weigh(*divmod(i, n_ck))
            yield top_log
        if hi < n_units * n_ck:
            u = hi // n_ck
            carry_v[0:8], carry_v[8:16] = maxima[u], tops[u + 1]
            carry_v[16:24], carry_v[24 : 24 + dh] = sums[u], accs[u]

    def projections(refs, wqkv_v, form_v, kept_v, ln_v):
        qt_v, k_v, vt_v = refs[:3]

        def normalise(base, ticks):
            zero = zero_s[0]
            centred = ln_v[base // LN_BATCH % len(ln_v)]
            rows = range(base, base + LN_BATCH, LN_ROWS)
            mean = [
                jnp.mean(x_v[i : i + LN_ROWS, :].astype(F32), axis=-1, keepdims=True)
                for i in rows
            ]
            mean = [_after(m, next(ticks)) for m in mean]
            scale = []
            for i, m in zip(rows, mean):
                again = pl.ds(pl.multiple_of(i + zero, LN_ROWS), LN_ROWS)
                x = x_v[again, :].astype(F32) - m
                var = jnp.mean(x * x, axis=-1, keepdims=True)
                scale.append(lax.rsqrt(var + LN_EPS))
                centred[zero, i - base : i - base + LN_ROWS, :] = x
            for i, g in zip(rows, scale):
                xn = centred[zero, i - base : i - base + LN_ROWS, :] * g
                r, row = divmod(i, ROWS)
                for n in range(n_grp):
                    a_v[r, n, row : row + LN_ROWS, :] = xn[:, n * LANES : (n + 1) * LANES]

        def copies(name):
            sem = start_sem.at[[name in names for names in _WAITS].index(True)]
            if name[0] == "x":
                rows = pl.ds(int(name[1:]) * X_PIECE, X_PIECE)
                yield pltpu.make_async_copy(x_hbm.at[rows], x_v.at[rows], sem)
                return
            r, lo, hi = map(int, name[1:])
            for mat in range(3):
                rows = pl.ds(r * D // 2, D // 2)
                cols = pl.ds(mat * D + lo * LANES, (hi - lo) * LANES)
                yield pltpu.make_async_copy(
                    wqkv_hbm.at[rows, cols], wqkv_v.at[rows, cols], sem
                )

        next_form, multiply = operands(form_v, lambda r, g: a_v[r, g, 0:ROWS, :], wqkv_v)
        count, latest = [0], [()]

        def product(o, s):
            left, right, *_ = _HK_ROW_BY_ROW[s]
            only_v = len(left) == 3
            a, result = multiply(o, left, right, [2] if only_v else range(3))
            for g in range(gpb):
                n = [terms for terms, *_ in _HK].index(left)
                xf_v[o * len(_HK) + n, g] = a[g].astype(BF16)
            count[0], latest[0] = count[0] + 1, result
            if only_v:
                return jnp.concatenate([jnp.zeros((ROWS, 2 * LANES), F32), result], axis=1)
            return result

        def amend(o, i, j, v):
            if (i, j) not in ((0, 3), (3, 0)):
                return v
            u0, u1 = (multiply(o, [(1, i, k)], [(1, j, 3 - k)], range(2))[1] for k in (1, 2))
            return jnp.concatenate([u0 + u1, v[:, 2 * LANES :]], axis=1)

        def emit(r, c, v):
            c = n_grp - 1 - c
            q, k, v = (v[:, n * LANES : (n + 1) * LANES] for n in range(3))
            q = q * (dh**-0.5 * math.log2(math.e))
            qt_v[c * n_qb + r] = _pack(q.astype(BF16).T)
            k_v[c, pl.ds(r * ROWS // 2, ROWS // 2), :] = _pack(k.astype(BF16))
            vt_v[c, :, pl.ds(r * ROWS, ROWS)] = _pack(v.astype(BF16).T)

        kept = temporaries(kept_v)
        ln_batches = iter(range(0, S, LN_BATCH))

        def do(work):
            latest[0] = ()
            for kind, group in itertools.groupby("".join(work)):
                n, after = len(list(group)), latest[0]
                if kind == "p":
                    todo = range(count[0], count[0] + n)
                    _block_product(product, emit, kept, todo, _HK_ROW_BY_ROW, amend)
                elif kind == "a":
                    _advance(attend(refs, None, 0, -n_ck - LAG, CUT, hpg))
                elif kind == "f":
                    for m in range(n):
                        col = len(after) and m * after.shape[1] // LANES // n * LANES
                        next_form(after[:, col : col + LANES] if len(after) else after)
                else:
                    rows = range(0, ROWS, ROWS * LN_ROWS // (n * LN_BATCH) // 8 * 8)
                    ticks = (after[i : i + LN_ROWS, :1] if len(after) else () for i in rows)
                    for base in itertools.islice(ln_batches, n):
                        normalise(base, ticks)

        for action, *names in _START_UP:
            if action == "do":
                do(names)
            elif action == "block":
                own_block(count[0])(lambda: do(names))
            else:
                for copy in itertools.chain(*map(copies, names)):
                    copy.start() if action == "start" else copy.wait()
        assert count[0] == N_PROD and next(ln_batches, None) is None

    def attention(refs, form_v, kept_v, wo_v, o_v):
        late = [
            pltpu.make_async_copy(wo_hbm, wo_v, late_sem),
            pltpu.make_async_copy(wd_hbm, wd_v, late_sem),
        ]
        for copy in (*late, *gate_up_copies(0)):
            copy.start()
        end = UNROLL * hpg * n_ck

        @pl.loop(0, n_step - UNROLL, step=UNROLL)
        def _(t):
            _advance(attend(refs, o_v, t, CUT, CUT + end, (UNROLL + 1) * hpg))

        for copy in late:
            copy.wait()
        next_form, multiply = operands(
            form_v, lambda r, g: o_v[(n_grp - 1 - g) * n_qb + r, 0:ROWS, :], wo_v
        )
        rest = attend(refs, o_v, n_step - UNROLL, CUT, end, UNROLL * hpg)
        for n in range(end - CUT - n_ck - LAG, 0, -1):
            tops = next(rest)
            if n % 16 == 1 and n < 16 * 4 * (gpb + 1):
                ticks = [t[:, :LANES] for t in tops[-16:] for _ in range(2)]
                next_form(jnp.concatenate(ticks, axis=0))

        def product(o, s):
            _advance(rest, int(_LAST_UNIT[s]))
            result = multiply(o, *_HK[s][:2], [0])[1]
            if _TWELVE_PIECES[s] == "1":
                next_form(result)
            return result

        def emit(r, c, v):
            a_v[r, c, 0:ROWS, :] = v

        own_block(0)(lambda: _block_product(product, emit, temporaries(kept_v)))

    def attention_branch(*refs):
        pl.run_scoped(
            functools.partial(projections, refs),
            pltpu.VMEM((D, 3 * D), BF16),
            [pltpu.VMEM((1, 12, gpb + 3, ROWS + PAD, LANES), F32)] * 2,
            _kept_shapes(3 * LANES),
            [pltpu.VMEM((1, LN_BATCH, D), F32)] * 16,
        )
        pl.run_scoped(
            functools.partial(attention, refs),
            [pltpu.VMEM((1, 12, gpb + 1, ROWS + PAD, LANES), F32)] * 2,
            _kept_shapes(LANES),
            pltpu.VMEM((D, D), BF16),
            pltpu.VMEM((n_step, ROWS + PAD, LANES), F32),
        )

    pl.run_scoped(
        attention_branch,
        pltpu.VMEM((n_step, LANES // 2, ROWS), U32),
        pltpu.VMEM((n_grp, S // 2, LANES), U32),
        pltpu.VMEM((n_grp, LANES // 2, S), U32),
        [pltpu.VMEM((S, ROWS), F32)] * 2,
        pltpu.VMEM((2 * dh, ROWS), F32),
    )

    def ffn_branch(h_v, down_v, form_v, kept_v):
        def down_forms(o, chunks, zero, offset=0):
            for i, j, part in itertools.product(range(4), chunks, range(3)):
                after = yield
                after = jnp.concatenate([after[r : r + 8] for r in range(0, ROWS, 16)], 0)
                rows = pl.ds(part * LANES, LANES)

                def h_block(k, r, c):
                    return h_v[1 - r][j + offset, 4 * i + 2 * c + k, rows, :]

                def wd_block(k, r, c):
                    first = pl.multiple_of(j * FC + (2 * r + k) * LANES, LANES)
                    return wd_v[pl.ds(first, LANES), pl.ds((4 * c + i) * LANES, LANES)]

                if part < 2:
                    forms = _left_forms(o, h_block, after)
                else:
                    forms = _right_forms(o, wd_block, after)
                for k, f in enumerate(forms):
                    down_v[o % 2][zero, j, 3 * i + k, rows, :] = f

        @pl.loop(0, n_fc)
        def _(j):
            @pl.when(j + 1 < n_fc)
            def _():
                for copy in gate_up_copies(j + 1):
                    copy.start()

            for copy in gate_up_copies(j):
                copy.wait()
            zero = zero_s[0]
            kept = temporaries(kept_v)
            gate, up = (
                jnp.max(jnp.abs(w_v[j % 2, n, 0:16, :].astype(F32)), keepdims=True)
                for n in range(2)
            )
            usable = jnp.minimum(gate, up) > 0
            ratio = jnp.where(usable, up, 1.0) / jnp.where(usable, gate, 1.0)
            ratio = jnp.clip(ratio * math.sqrt(2), 2.0**-30, 2.0**30)
            ratio = lax.bitcast_convert_type(ratio, jnp.int32) & 0x7F800000
            ratio = lax.bitcast_convert_type(ratio, F32)
            half_inverse = 0.5 / ratio

            def form(o, i, k):
                return form_v[(o % 2 * 4 + i) * 3 + k].at[zero]

            def prepare(o, i, after=()):
                def block(k, r, c):
                    rows, cols = pl.ds((2 * r + k) * kb, kb), pl.ds(i * LANES, LANES)
                    w = w_v[j % 2, c, rows, cols].astype(F32)
                    return w if c else w * ratio

                for k, f in enumerate(_right_forms(o, block, after)):
                    form(o, i, k)[...] = f

            def product(o, s):
                a = [xf_v.bitcast(U32)[o * len(_HK) + s, g] for g in range(gpb)]
                if o == 0 and s < 2:
                    assert _HK[s][1] == [(1, 1 + s, 0)]
                    w = w_v[j % 2, 1, pl.ds(3 * kb, kb), pl.ds((1 + s) * LANES, LANES)]
                else:
                    w = _signed_sum(_HK[s][1], lambda i, k: form(o, i, k)[...])
                result = _dot(jnp.concatenate(list(map(_unpack, a)), 1), w.astype(BF16))
                if o == 0 and s in (0, 5):
                    prepare(0, 2 + (0, 5).index(s), result)
                if o < 6 and s in (2, 9, 13, 17):
                    prepare(o + 1, (2, 9, 13, 17).index(s), result)
                if o == 6 and _TWELVE_PIECES[s] == "1":
                    first_down_forms(result)
                return result

            def emit(r, c, v):
                if c < 4:
                    v = 0.5 * jnp.tanh(v * half_inverse) + 0.5
                other = kept[1][4 * (r % 4) + c % 4][5 if r < 4 else 0]
                if (r < 4) != (c < 4):
                    other[...] = v
                else:
                    h_v[r // 4][j, 4 * (r % 4) + c % 4, 0:ROWS, :] = v * other[...]

            first_down_forms = _paced(down_forms(0, [j], zero, zero))
            prepare(0, 0)
            prepare(0, 1)
            _block_product(product, emit, kept)
            assert first_down_forms(None)

        zero = zero_s[0]
        following = [_paced(down_forms(o, range(n_fc), zero)) for o in range(1, 7)]

        def product(o, s):
            def form(rows, j, i, k):
                return down_v[o % 2][zero, j, 3 * i + k, rows, :]

            parts = []
            for js in (range(0, 4), range(4, n_fc)):
                a, w = (
                    [_signed_sum(terms, functools.partial(form, rows, j)) for j in js]
                    for terms, rows in zip(_HK[s], (pl.ds(0, ROWS), pl.ds(ROWS, LANES)))
                )
                a, w = jnp.concatenate(a, axis=1), jnp.concatenate(w, axis=0)
                parts.append(_dot(a.astype(BF16), w.astype(BF16)))
            if o < 6:
                count = int(_DOWN_PIECES[s])
                for n in range(count):
                    following[o](parts[2 * n // count])
                assert s + 1 < len(_HK) or following[o](None)
            return parts[0] + parts[1]

        done, out_copies = [], []

        def emit(r, c, d):
            r = (r + 4) % 8
            rows, cols = pl.ds(r * ROWS, ROWS), pl.ds(c * LANES, LANES)
            silu = d * (0.5 * jnp.tanh(0.5 * d) + 0.5)
            y = x_v[rows, cols].astype(F32) + a_v[r, c, 0:ROWS, :] * silu
            x_v[rows, cols] = y.astype(x_v.dtype)
            done.append((r, c))
            width = 1 if len(done) > 48 else 4
            c = c // width * width
            if all((r, c + n) in done for n in range(width)):
                cols = pl.ds(c * LANES, width * LANES)
                out_copies.append(
                    pltpu.make_async_copy(
                        x_v.at[rows, cols], out_hbm.at[rows, cols], out_sem
                    )
                )
                out_copies[-1].start()

        kept = temporaries(kept_v)
        for lo, hi in itertools.pairwise((0, 45, 89, 136, N_PROD)):
            own_block(lo)(lambda: _block_product(product, emit, kept, range(lo, hi)))
        for copy in out_copies:
            copy.wait()

    pl.run_scoped(
        ffn_branch,
        [pltpu.VMEM((n_fc, 16, ROWS + PAD, LANES), F32)] * 2,
        [pltpu.VMEM((1, n_fc, 12, ROWS + LANES + PAD, LANES), F32)] * 2,
        [pltpu.VMEM((1, kb, LANES), F32)] * 24,
        _kept_shapes(LANES, slots=6),
    )


@jax.jit
def pallas_recurrent_scan__softmax_full_mha__glu_gated_glu__prompt_kernel(
    A_x: jax.Array,
    A_wqkv: jax.Array,
    A_wo: jax.Array,
    B_x: jax.Array,
    B_w_gate: jax.Array,
    B_w_up: jax.Array,
    B_w_down: jax.Array,
):
    del B_x
    B, S, D = A_x.shape
    F = B_w_gate.shape[1]
    assert (B, S, D, F) == (1, 2048, 1024, 3584)

    out = pl.pallas_call(
        _kernel,
        out_shape=jax.ShapeDtypeStruct((S, D), A_x.dtype),
        in_specs=[pl.BlockSpec(memory_space=pl.ANY)] * 6,
        out_specs=pl.BlockSpec(memory_space=pl.ANY),
        scratch_shapes=[
            pltpu.VMEM((S, D), A_x.dtype),
            pltpu.VMEM((2, 2, D, FC), BF16),
            pltpu.VMEM((F, D), BF16),
            pltpu.VMEM((N_PROD, 2, ROWS, LANES), BF16),
            pltpu.VMEM((S // ROWS, D // LANES, ROWS + PAD, LANES), F32),
            pltpu.SMEM((1,), jnp.int32),
            pltpu.SemaphoreType.DMA((len(_WAITS),)),
            pltpu.SemaphoreType.DMA((2,)),
            pltpu.SemaphoreType.DMA(()),
            pltpu.SemaphoreType.DMA(()),
        ],
        compiler_params=pltpu.CompilerParams(vmem_limit_bytes=127 * 2**20),
    )(A_x.reshape(S, D), A_wqkv, A_wo, B_w_gate, B_w_up, B_w_down)
    return out.reshape(B, S, D)
```

```python
import functools
import itertools
import math

import jax
import jax.numpy as jnp
from jax import lax
import jax.experimental.pallas as pl
import jax.experimental.pallas.tpu as pltpu

F32 = jnp.float32
BF16 = jnp.bfloat16
U32 = jnp.uint32

N_HEADS = 32
LN_EPS = 1e-5
LANES = 128
ROWS = 256
FC = 4 * LANES
PAD = 8

CK = 128
LAG = 4
CUT = 8
UNROLL = 4
VPU_CHUNKS = (10, 11)
EXP_PACE, KEY_PACE, SUM_PACE = 7, 5, 9

X_PIECE = 128
LN_BATCH = 32
LN_ROWS = 16

_START_UP = [
    line.split()
    for line in """
start x0 x1
wait x0
do nnnn
start w145
wait x1
do nnnn ff
start x2 x3
wait w145
do fff pp
start w156
wait x2 x3
do nnnnnnnn ff
start x4 x5
wait w156
do fff ppp
start w167
wait x4 x5
do nnn pnnnnn pff
start x6 x7
wait w167
do fff ppp
start w178 w046
wait x6 x7
do nn pnn pnn pnn f p f
start w068 x8 x9 x10 x11
wait w178 w046
do fff pf pf pf pff pf pf pf pf pf ppp
start x12 x13 x14 x15 w004
wait w068 x8 x9 x10 x11
do f pf pf pf pfn pnn pn pn pffn pffn pfn pn pn p
start w104
wait x12 x13 x14 x15 w004
do f pf pf pffnn pnn pnn pff pf pf pf pnn pn pn p pnn pnn pffn pffn pfnn pnn pnn p
wait w104
block f pff pff pf pf pff pf pf pff pff pff pff pf pf pf pff pf pp {forms}
block ppppppp {forms} ppppppp pff pf pff pff pf p p pff pff
block pf p p pff p p pff pff p pf ppppppp pppppppppppppppppppppppppp a
""".format(forms="pff pf pff pff pf p p pff pff pf p p pff p p pff pff p pf")
    .strip()
    .split("\n")
]
_WAITS = [names for action, *names in _START_UP if action == "wait"]
_TWELVE_PIECES = "11101110011001000110001000"
_LAST_UNIT = "10101011010110110101101100"
_DOWN_PIECES = "44444443344334343443333321"
_FINISH_PIECES = "22222121122112121111010100"

_A_TERMS = (
    ((1, 0, 0), (1, 0, 1)),
    ((1, 0, 0),),
    ((1, 1, 0), (1, 1, 1)),
    ((1, 1, 1),),
    ((1, 0, 0), (1, 1, 1)),
    ((1, 1, 0), (-1, 0, 0)),
    ((1, 0, 1), (-1, 1, 1)),
)
_B_TERMS = (
    ((1, 1, 1),),
    ((1, 0, 1), (-1, 1, 1)),
    ((1, 0, 0),),
    ((1, 1, 0), (-1, 0, 0)),
    ((1, 0, 0), (1, 1, 1)),
    ((1, 0, 0), (1, 0, 1)),
    ((1, 1, 0), (1, 1, 1)),
)


def _strassen_combine(k, v, slots):
    if k in (0, 1, 2, 4):
        slots[k][...] = v
    if k == 1:
        return 0, 1, slots[0][...] + v
    if k == 3:
        slots[3][...] = v - slots[0][...]
        return 1, 0, slots[2][...] + v
    if k == 5:
        return 1, 1, slots[1][...] - slots[2][...] + slots[4][...] + v
    if k == 6:
        return 0, 0, slots[3][...] + slots[4][...] + v
    return None


def _signed_sum(terms, block):
    assert terms[0][0] == 1
    acc = None
    for sign, *key in terms:
        b = block(*key).astype(F32)
        acc = b if acc is None else (acc + b if sign > 0 else acc - b)
    return acc


def _after(x, y):
    return jnp.minimum(x, jnp.maximum(x, y)) if len(y) else x


def _left_forms(o, block, after):
    a0, a1 = (_signed_sum(_A_TERMS[o], functools.partial(block, k)) for k in range(2))
    a0 = _after(a0, after)
    h = -0.5 * a0
    return a0, a1 + h, a1 - h


def _right_forms(o, block, after):
    b0, b1 = (_signed_sum(_B_TERMS[o], functools.partial(block, k)) for k in range(2))
    b1 = _after(b1, after)
    h = 0.5 * b1
    return b1, h + b0, h - b0


def _hopcroft_kerr(order):
    t_of = (0, 1, 2, 0, 2)

    def left(sign, i, k):
        sign = sign if k < 2 else -sign
        return [(sign, i, k)] if i < 4 else [(sign, 0, k), (-sign, 1, k)]

    def right(sign, j, k):
        sign = sign if k else -sign
        return [(sign, j, k)] if j < 4 else [(sign, 0, k), (sign, 1, k)]

    def diagonal(i):
        l, m = (t_of[i] + 1) % 3, (t_of[i] + 2) % 3
        u = left(1, i, l), right(1, i, m), f"u{i}"
        v = left(1, i, m), right(1, i, l), f"v{i}"
        yield *(u if l else v), None
        yield *(v if l else u), (i, i, [(1, f"u{i}"), (-1, f"v{i}")], None)

    def pair(i, j, names=("p", "q"), row=None, more=((), ())):
        k, l, m, r = t_of[i], t_of[j], f"m{i}{j}", i if row is None else row
        assert l == (k + 1) % 3
        upper = [(1, f"v{i}"), (-1, f"v{j}"), *more[0], (1, m), (1, names[0])]
        lower = [(1, f"u{i}"), (-1, f"u{j}"), *more[1], (1, m), (1, names[1])]
        yield left(1, i, l) + left(1, j, k), right(1, i, l) + right(-1, j, k), m, None
        yield (
            left(1, i, k) + left(-1, j, k), right(1, i, l) + right(1, j, l),
            names[0], (r, j, upper, f"c{r}{j}"),
        )
        yield (
            left(1, i, l) + left(-1, j, l), right(1, i, k) + right(1, j, k),
            names[1], (j, r, lower, f"c{j}{r}"),
        )

    groups = {str(i): diagonal(i) for i in range(4)}
    groups.update({f"{i}{j}": pair(i, j) for i, j in ((1, 2), (2, 0), (3, 1), (2, 3))})
    groups["01"] = pair(0, 1, names=("u4", "v4"))
    groups["43"] = pair(4, 3, row=0, more=([(1, "c13")], [(-1, "c31")]))

    def plus_first(terms):
        n = [sign for sign, *_ in terms].index(1)
        return [terms[n]] + terms[:n] + terms[n + 1 :]

    steps, signs = [], {}
    for a, b, name, result in (next(groups[g]) for g in order.split()):
        flips = [max(sign for sign, *_ in terms) for terms in (a, b)]
        a, b = (
            plus_first([(sign * flip, *key) for sign, *key in terms])
            for terms, flip in zip((a, b), flips)
        )
        signs[name] = flips[0] * flips[1]
        if result is not None:
            i, j, terms, c = result
            result = i, j, plus_first([(s * signs.get(n, 1), n) for s, n in terms]), c
        steps.append((a, b, name, result))
    return steps


_HK = _hopcroft_kerr(
    "1 2 0 1 0 01 2 01 01 12 20 12 12 3 20 3 20 31 23 31 31 23 43 23 43 43"
)
_HK_ROW_BY_ROW = _hopcroft_kerr(
    "0 0 1 01 1 01 01 2 12 2 12 12 20 20 20 3 31 3 23 31 31 23 43 23 43 43"
)
_HK_KEPT = sorted(
    {n for *_, name, result in _HK if result for _, n in result[2] if n != name}
)
N_PROD = 7 * len(_HK)


def _block_product(product, emit, kept, products=range(N_PROD), steps=_HK, amend=None):
    inner, outer = dict(zip(_HK_KEPT, kept[0])), kept[1]
    for number in products:
        o, s = divmod(number, len(steps))
        *_, name, result = steps[s]
        v = product(o, s)
        if name in inner:
            inner[name][...] = v
        if result is None:
            continue
        i, j, terms, c = result
        v = _signed_sum(terms, lambda n: v if n == name else inner[n][...])
        if c in inner:
            inner[c][...] = v
        if amend is not None:
            v = amend(o, i, j, v)
        done = _strassen_combine(o, v, outer[4 * i + j])
        if done is not None:
            emit(4 * done[0] + i, 4 * done[1] + j, done[2])


def _kept_shapes(width, slots=5):
    block = pltpu.VMEM((1, ROWS, width), F32)
    return [block] * len(_HK_KEPT), [[block] * slots] * 16


def _advance(work, count=None):
    for _ in itertools.islice(work, count):
        pass


def _paced(work):
    next(work)
    left = [True]

    def step(y):
        if left and y is not None:
            try:
                work.send(y)
            except StopIteration:
                left.clear()
        return not left

    return step


def _pack(x):
    return pltpu.bitcast(x, U32)


def _unpack(x):
    return pltpu.bitcast(x, BF16)


def _dot(a, b):
    return jnp.dot(a, b, preferred_element_type=F32)


def _fold_rows(op, x):
    r = x[0:8]
    for i in range(1, x.shape[0] // 8):
        r = op(r, x[8 * i : 8 * i + 8])
    return r


def _kernel(
    x_hbm, wqkv_hbm, wo_hbm, wg_hbm, wu_hbm, wd_hbm, out_hbm,
    x_v, w_v, wd_v, xf_v, a_v, zero_s,
    start_sem, w_sem, late_sem, out_sem,
):
    S, D = x_v.shape
    n_fc = wd_v.shape[0] // FC
    kb = D // 4
    dh = D // N_HEADS
    hpg = LANES // dh
    n_grp, gpb = D // LANES, kb // LANES
    n_qb = S // ROWS

    zero_s[0] = 0

    def temporaries(refs):
        zero = zero_s[0]
        return [t.at[zero] for t in refs[0]], [[t.at[zero] for t in r] for r in refs[1]]

    def own_block(n):
        return pl.when(zero_s[0] <= n)

    def gate_up_copies(j):
        cols = pl.ds(pl.multiple_of(j * FC, FC), FC)
        for n, src in enumerate((wg_hbm, wu_hbm)):
            yield pltpu.make_async_copy(src.at[:, cols], w_v.at[j % 2, n], w_sem.at[j % 2])

    def operands(form_v, left_block, weights):
        zero = zero_s[0]
        n_part = gpb + weights.shape[1] // D
        ready, in_use = [], [0]

        def make_forms():
            for o, i, part in itertools.product(range(7), range(4), range(n_part)):
                after = yield
                assert in_use[0] >= o - 1

                def a_block(k, r, c):
                    return left_block(4 * r + i, (2 * c + k) * gpb + part)

                def w_block(k, r, c):
                    col = (part - gpb) * D + (4 * c + i) * LANES
                    return weights[pl.ds((2 * r + k) * kb, kb), pl.ds(col, LANES)]

                if part < gpb:
                    forms = _left_forms(o, a_block, after)
                else:
                    forms = _right_forms(o, w_block, after)
                for k, f in enumerate(forms):
                    form_v[o % 2][zero, 3 * i + k, part, 0:ROWS, :] = f
                ready.append((o, i, part))

        def multiply(o, left, right, mats):
            in_use[0] = o

            def form(part, i, k):
                assert (o, i, part) in ready
                return form_v[o % 2][zero, 3 * i + k, part, 0:ROWS, :]

            a, w = (
                [_signed_sum(terms, functools.partial(form, part)) for part in parts]
                for terms, parts in ((left, range(gpb)), (right, [gpb + m for m in mats]))
            )
            a, w = (jnp.concatenate(x, axis=1).astype(BF16) for x in (a, w))
            return a, _dot(a, w)

        return _paced(make_forms()), multiply

    n_ck = S // CK
    n_step = n_grp * n_qb

    def attend(refs, o_v, t, lo, hi, n_units):
        qt_v, k_v, vt_v, sc_v, carry_v = refs
        queries, maxima, tops, sums, accs = {}, {}, {}, {}, {}
        top_log, partial, outs = [], [], []
        if lo > 0:
            maxima[0], tops[1] = carry_v[0:8], carry_v[8:16]
            sums[0], accs[0] = carry_v[16:24], carry_v[24 : 24 + dh]

        def score_on_vpu(u, c):
            step, h = t + u // hpg, u % hpg
            j, d0 = divmod(8 * c, dh)
            q = _unpack(qt_v[step, pl.ds((h * dh + d0) // 16 * 8, 8), :]).astype(F32)
            q = q[d0 % 16 : d0 % 16 + 8]
            if len(partial) >= SUM_PACE:
                q = _after(q, partial[-SUM_PACE])
            row = (VPU_CHUNKS[j // 2] + 1) * CK - 16
            k = _unpack(k_v[step // n_qb, pl.ds(row // 2, 8), :]).astype(F32)
            k, row = k[j % 2 * 8 : j % 2 * 8 + 8], row + j % 2 * 8
            if len(top_log) >= KEY_PACE:
                k = _after(k, top_log[-KEY_PACE][:, :LANES])
            for d in range(8):
                lane = h * dh + d0 + d
                term = k[:, lane : lane + 1] * q[d : d + 1]
                partial.append(partial[-1] + term if d0 + d else term)
            if d0 + 8 == dh:
                sc_v[u % 2][row : row + 8, :] = partial[-1]
                tops[u] = jnp.maximum(tops[u], partial[-1])

        def score(u, c):
            step, h = t + u // hpg, u % hpg
            if u not in queries:
                r0, r1 = h * dh // 2, (h + 1) * dh // 2
                parts = [qt_v[step, r0:r1, :]]
                if r0:
                    parts.insert(0, jnp.zeros((r0, ROWS), U32))
                if r1 < LANES // 2:
                    parts.append(jnp.zeros((LANES // 2 - r1, ROWS), U32))
                queries[u] = _unpack(jnp.concatenate(parts, axis=0))
            n = CK - 16 * (c in VPU_CHUNKS)
            k = k_v[step // n_qb, pl.ds(c * CK // 2, n // 2), :]
            s = _dot(_unpack(k), queries[u])
            sc_v[u % 2][pl.ds(c * CK, n), :] = s
            top = _fold_rows(jnp.maximum, s)
            tops[u] = jnp.maximum(tops[u], top) if c else top
            top_log.append(tops[u])
            score_on_vpu(u, c)
            if c == n_ck - 1:
                m = jnp.max(tops[u], axis=0, keepdims=True)
                maxima[u] = jnp.broadcast_to(m, (8, ROWS))

        def weigh(u, c):
            step, h = t + u // hpg, u % hpg
            m = maxima[u]
            if len(top_log) >= EXP_PACE:
                m = _after(m, top_log[-EXP_PACE])
            keys = slice(c * CK, (c + 1) * CK)
            p = jnp.exp2(sc_v[u % 2][keys, :] - jnp.tile(m, (CK // 8, 1)))
            total = _fold_rows(jnp.add, p)
            sums[u] = sums[u] + total if c else total
            vt = vt_v[step // n_qb, h * dh // 2 : (h + 1) * dh // 2, keys]
            o = _dot(_unpack(vt), p.astype(BF16))
            accs[u] = accs[u] + o if c else o
            if c == n_ck - 1:
                total = jnp.sum(sums[u], axis=0, keepdims=True)
                outs.append(accs[u] * (1.0 / total))
                if h == hpg - 1:
                    o_v[step, 0:ROWS, :] = jnp.concatenate(outs[-hpg:], axis=0).T

        for i in range(lo, hi):
            ahead = i + n_ck + LAG
            if ahead < n_units * n_ck:
                score(*divmod(ahead, n_ck))
            if i >= 0:
                weigh(*divmod(i, n_ck))
            yield top_log
        if hi < n_units * n_ck:
            u = hi // n_ck
            carry_v[0:8], carry_v[8:16] = maxima[u], tops[u + 1]
            carry_v[16:24], carry_v[24 : 24 + dh] = sums[u], accs[u]

    def projections(refs, wqkv_v, form_v, kept_v, ln_v):
        qt_v, k_v, vt_v = refs[:3]

        def normalise(base, ticks):
            zero = zero_s[0]
            centred = ln_v[base // LN_BATCH % len(ln_v)]
            rows = range(base, base + LN_BATCH, LN_ROWS)
            mean = [
                jnp.mean(x_v[i : i + LN_ROWS, :].astype(F32), axis=-1, keepdims=True)
                for i in rows
            ]
            mean = [_after(m, next(ticks)) for m in mean]
            scale = []
            for i, m in zip(rows, mean):
                again = pl.ds(pl.multiple_of(i + zero, LN_ROWS), LN_ROWS)
                x = x_v[again, :].astype(F32) - m
                var = jnp.mean(x * x, axis=-1, keepdims=True)
                scale.append(lax.rsqrt(var + LN_EPS))
                centred[zero, i - base : i - base + LN_ROWS, :] = x
            for i, g in zip(rows, scale):
                xn = centred[zero, i - base : i - base + LN_ROWS, :] * g
                r, row = divmod(i, ROWS)
                for n in range(n_grp):
                    a_v[r, n, row : row + LN_ROWS, :] = xn[:, n * LANES : (n + 1) * LANES]

        def copies(name):
            sem = start_sem.at[[name in names for names in _WAITS].index(True)]
            if name[0] == "x":
                rows = pl.ds(int(name[1:]) * X_PIECE, X_PIECE)
                yield pltpu.make_async_copy(x_hbm.at[rows], x_v.at[rows], sem)
                return
            r, lo, hi = map(int, name[1:])
            for mat in range(3):
                rows = pl.ds(r * D // 2, D // 2)
                cols = pl.ds(mat * D + lo * LANES, (hi - lo) * LANES)
                yield pltpu.make_async_copy(
                    wqkv_hbm.at[rows, cols], wqkv_v.at[rows, cols], sem
                )

        next_form, multiply = operands(form_v, lambda r, g: a_v[r, g, 0:ROWS, :], wqkv_v)
        count, latest = [0], [()]

        def product(o, s):
            left, right, *_ = _HK_ROW_BY_ROW[s]
            only_v = len(left) == 3
            a, result = multiply(o, left, right, [2] if only_v else range(3))
            xf_v[o * len(_HK) + [terms for terms, *_ in _HK].index(left)] = _pack(a)
            count[0], latest[0] = count[0] + 1, result
            if only_v:
                return jnp.concatenate([jnp.zeros((ROWS, 2 * LANES), F32), result], axis=1)
            return result

        def amend(o, i, j, v):
            if (i, j) not in ((0, 3), (3, 0)):
                return v
            u0, u1 = (multiply(o, [(1, i, k)], [(1, j, 3 - k)], range(2))[1] for k in (1, 2))
            return jnp.concatenate([u0 + u1, v[:, 2 * LANES :]], axis=1)

        def emit(r, c, v):
            c = n_grp - 1 - c
            q, k, v = (v[:, n * LANES : (n + 1) * LANES] for n in range(3))
            q = q * (dh**-0.5 * math.log2(math.e))
            qt_v[c * n_qb + r] = _pack(q.astype(BF16).T)
            k_v[c, pl.ds(r * ROWS // 2, ROWS // 2), :] = _pack(k.astype(BF16))
            vt_v[c, :, pl.ds(r * ROWS, ROWS)] = _pack(v.astype(BF16).T)

        kept = temporaries(kept_v)
        ln_batches = iter(range(0, S, LN_BATCH))

        def do(work):
            latest[0] = ()
            for kind, group in itertools.groupby("".join(work)):
                n, after = len(list(group)), latest[0]
                if kind == "p":
                    todo = range(count[0], count[0] + n)
                    _block_product(product, emit, kept, todo, _HK_ROW_BY_ROW, amend)
                elif kind == "a":
                    _advance(attend(refs, None, 0, -n_ck - LAG, CUT, hpg))
                elif kind == "f":
                    for m in range(n):
                        col = len(after) and m * after.shape[1] // LANES // n * LANES
                        next_form(after[:, col : col + LANES] if len(after) else after)
                else:
                    rows = range(0, ROWS, ROWS * LN_ROWS // (n * LN_BATCH) // 8 * 8)
                    ticks = (after[i : i + LN_ROWS, :1] if len(after) else () for i in rows)
                    for base in itertools.islice(ln_batches, n):
                        normalise(base, ticks)

        for action, *names in _START_UP:
            if action == "do":
                do(names)
            elif action == "block":
                own_block(count[0])(lambda: do(names))
            else:
                for copy in itertools.chain(*map(copies, names)):
                    copy.start() if action == "start" else copy.wait()
        assert count[0] == N_PROD and next(ln_batches, None) is None

    def attention(refs, form_v, kept_v, wo_v, o_v):
        late = [
            pltpu.make_async_copy(wo_hbm, wo_v, late_sem),
            pltpu.make_async_copy(wd_hbm, wd_v, late_sem),
        ]
        for copy in (*late, *gate_up_copies(0)):
            copy.start()
        end = UNROLL * hpg * n_ck

        @pl.loop(0, n_step - UNROLL, step=UNROLL)
        def _(t):
            _advance(attend(refs, o_v, t, CUT, CUT + end, (UNROLL + 1) * hpg))

        for copy in late:
            copy.wait()
        next_form, multiply = operands(
            form_v, lambda r, g: o_v[(n_grp - 1 - g) * n_qb + r, 0:ROWS, :], wo_v
        )
        rest = attend(refs, o_v, n_step - UNROLL, CUT, end, UNROLL * hpg)
        for n in range(end - CUT - n_ck - LAG, 0, -1):
            tops = next(rest)
            if n % 16 == 1 and n < 16 * 4 * (gpb + 1):
                ticks = [t[:, :LANES] for t in tops[-16:] for _ in range(2)]
                next_form(jnp.concatenate(ticks, axis=0))

        def product(o, s):
            _advance(rest, int(_LAST_UNIT[s]))
            result = multiply(o, *_HK[s][:2], [0])[1]
            if _TWELVE_PIECES[s] == "1":
                next_form(result)
            return result

        def emit(r, c, v):
            a_v[r, c, 0:ROWS, :] = v

        own_block(0)(lambda: _block_product(product, emit, temporaries(kept_v)))

    def attention_branch(*refs):
        pl.run_scoped(
            functools.partial(projections, refs),
            pltpu.VMEM((D, 3 * D), BF16),
            [pltpu.VMEM((1, 12, gpb + 3, ROWS + PAD, LANES), F32)] * 2,
            _kept_shapes(3 * LANES),
            [pltpu.VMEM((1, LN_BATCH, D), F32)] * 16,
        )
        pl.run_scoped(
            functools.partial(attention, refs),
            [pltpu.VMEM((1, 12, gpb + 1, ROWS + PAD, LANES), F32)] * 2,
            _kept_shapes(LANES),
            pltpu.VMEM((D, D), BF16),
            pltpu.VMEM((n_step, ROWS + PAD, LANES), F32),
        )

    pl.run_scoped(
        attention_branch,
        pltpu.VMEM((n_step, LANES // 2, ROWS), U32),
        pltpu.VMEM((n_grp, S // 2, LANES), U32),
        pltpu.VMEM((n_grp, LANES // 2, S), U32),
        [pltpu.VMEM((S, ROWS), F32)] * 2,
        pltpu.VMEM((2 * dh, ROWS), F32),
    )

    def ffn_branch(h_v, down_v, form_v, kept_v):
        def down_forms(o, chunks, zero, offset=0):
            for i, j, part in itertools.product(range(4), chunks, range(3)):
                after = yield
                after = jnp.concatenate([after[r : r + 8] for r in range(0, ROWS, 16)], 0)
                rows = pl.ds(part * LANES, LANES)

                def h_block(k, r, c):
                    return h_v[1 - r][j + offset, 4 * i + 2 * c + k, rows, :]

                def wd_block(k, r, c):
                    first = pl.multiple_of(j * FC + (2 * r + k) * LANES, LANES)
                    return wd_v[pl.ds(first, LANES), pl.ds((4 * c + i) * LANES, LANES)]

                if part < 2:
                    forms = _left_forms(o, h_block, after)
                else:
                    forms = _right_forms(o, wd_block, after)
                for k, f in enumerate(forms):
                    down_v[o % 2][zero, j, 3 * i + k, rows, :] = f

        @pl.loop(0, n_fc)
        def _(j):
            @pl.when(j + 1 < n_fc)
            def _():
                for copy in gate_up_copies(j + 1):
                    copy.start()

            for copy in gate_up_copies(j):
                copy.wait()
            zero = zero_s[0]
            kept = temporaries(kept_v)
            gate, up = (
                jnp.max(jnp.abs(w_v[j % 2, n, 0:16, :].astype(F32)), keepdims=True)
                for n in range(2)
            )
            usable = jnp.minimum(gate, up) > 0
            ratio = jnp.where(usable, up, 1.0) / jnp.where(usable, gate, 1.0)
            ratio = jnp.clip(ratio * math.sqrt(2), 2.0**-30, 2.0**30)
            ratio = lax.bitcast_convert_type(ratio, jnp.int32) & 0x7F800000
            ratio = lax.bitcast_convert_type(ratio, F32)
            half_inverse = 0.5 / ratio

            def form(o, i, k):
                return form_v[(o % 2 * 4 + i) * 3 + k].at[zero]

            def prepare(o, i, after=()):
                def block(k, r, c):
                    rows, cols = pl.ds((2 * r + k) * kb, kb), pl.ds(i * LANES, LANES)
                    w = w_v[j % 2, c, rows, cols].astype(F32)
                    return w if c else w * ratio

                for k, f in enumerate(_right_forms(o, block, after)):
                    form(o, i, k)[...] = f

            def product(o, s):
                if o == 0 and s < 2:
                    assert _HK[s][1] == [(1, 1 + s, 0)]
                    w = w_v[j % 2, 1, pl.ds(3 * kb, kb), pl.ds((1 + s) * LANES, LANES)]
                else:
                    w = _signed_sum(_HK[s][1], lambda i, k: form(o, i, k)[...])
                result = _dot(_unpack(xf_v[o * len(_HK) + s]), w.astype(BF16))
                if o == 0 and s in (0, 5):
                    prepare(0, 2 + (0, 5).index(s), result)
                if o < 6 and s in (2, 9, 13, 17):
                    prepare(o + 1, (2, 9, 13, 17).index(s), result)
                if o == 6 and _TWELVE_PIECES[s] == "1":
                    first_down_forms(result)
                return result

            def emit(r, c, v):
                if c < 4:
                    v = 0.5 * jnp.tanh(v * half_inverse) + 0.5
                other = kept[1][4 * (r % 4) + c % 4][5 if r < 4 else 0]
                if (r < 4) != (c < 4):
                    other[...] = v
                else:
                    h_v[r // 4][j, 4 * (r % 4) + c % 4, 0:ROWS, :] = v * other[...]

            first_down_forms = _paced(down_forms(0, [j], zero, zero))
            prepare(0, 0)
            prepare(0, 1)
            _block_product(product, emit, kept)
            assert first_down_forms(None)

        zero = zero_s[0]
        following = [_paced(down_forms(o, range(n_fc), zero)) for o in range(1, 7)]

        def product(o, s):
            def form(rows, j, i, k):
                return down_v[o % 2][zero, j, 3 * i + k, rows, :]

            parts = []
            for js in (range(0, 4), range(4, n_fc)):
                a, w = (
                    [_signed_sum(terms, functools.partial(form, rows, j)) for j in js]
                    for terms, rows in zip(_HK[s], (pl.ds(0, ROWS), pl.ds(ROWS, LANES)))
                )
                a, w = jnp.concatenate(a, axis=1), jnp.concatenate(w, axis=0)
                parts.append(_dot(a.astype(BF16), w.astype(BF16)))
            if o < 6:
                count = int(_DOWN_PIECES[s])
                for n in range(count):
                    following[o](parts[2 * n // count])
                assert s + 1 < len(_HK) or following[o](None)
            for n in range(int(_FINISH_PIECES[s]) if o in (2, 4, 6) else 0):
                finishing(parts[1 - n % 2])
            return parts[0] + parts[1]

        done, out_copies = [], []

        def finish(r, c, d, row=0):
            rows = pl.ds(r * ROWS + row, d.shape[0])
            blocks = range(c, c + d.shape[1] // LANES)
            cols = pl.ds(c * LANES, d.shape[1])
            s = jnp.concatenate([a_v[r, n, row : row + d.shape[0], :] for n in blocks], 1)
            y = x_v[rows, cols].astype(F32) + s * (d * (0.5 * jnp.tanh(0.5 * d) + 0.5))
            x_v[rows, cols] = y.astype(x_v.dtype)
            if row + d.shape[0] == ROWS:
                rows = pl.ds(r * ROWS, ROWS)
                out_copies.append(
                    pltpu.make_async_copy(
                        x_v.at[rows, cols], out_hbm.at[rows, cols], out_sem
                    )
                )
                out_copies[-1].start()
                done.extend((r, n) for n in blocks)

        waiting = {}

        def emit(r, c, d):
            if r < 4 and c < 4:
                finish((r + 4) % 8, c, d)
            else:
                waiting[(r + 4) % 8, c] = kept[1][4 * (r % 4) + c % 4][5]
                waiting[(r + 4) % 8, c][...] = d

        def finish_waiting():
            for _, row in itertools.product(range(24), range(0, ROWS, 64)):
                after = yield
                after = jnp.concatenate([after[n : n + 8] for n in range(0, ROWS, 32)], 0)
                r, c = min(k for k in waiting if k not in done)
                d = [_after(waiting[r, c + n][row : row + 64, :], after) for n in range(2)]
                finish(r, c, jnp.concatenate(d, axis=1), row)

        finishing = _paced(finish_waiting())
        kept = temporaries(kept_v)
        for lo, hi in itertools.pairwise((0, 45, 89, 136, N_PROD)):
            own_block(lo)(lambda: _block_product(product, emit, kept, range(lo, hi)))
        assert len(done) == 64
        for copy in out_copies:
            copy.wait()

    pl.run_scoped(
        ffn_branch,
        [pltpu.VMEM((n_fc, 16, ROWS + PAD, LANES), F32)] * 2,
        [pltpu.VMEM((1, n_fc, 12, ROWS + LANES + PAD, LANES), F32)] * 2,
        [pltpu.VMEM((1, kb, LANES), F32)] * 24,
        _kept_shapes(LANES, slots=6),
    )


@jax.jit
def pallas_recurrent_scan__softmax_full_mha__glu_gated_glu__prompt_kernel(
    A_x: jax.Array,
    A_wqkv: jax.Array,
    A_wo: jax.Array,
    B_x: jax.Array,
    B_w_gate: jax.Array,
    B_w_up: jax.Array,
    B_w_down: jax.Array,
):
    del B_x
    B, S, D = A_x.shape
    F = B_w_gate.shape[1]
    assert (B, S, D, F) == (1, 2048, 1024, 3584)

    out = pl.pallas_call(
        _kernel,
        out_shape=jax.ShapeDtypeStruct((S, D), A_x.dtype),
        in_specs=[pl.BlockSpec(memory_space=pl.ANY)] * 6,
        out_specs=pl.BlockSpec(memory_space=pl.ANY),
        scratch_shapes=[
            pltpu.VMEM((S, D), A_x.dtype),
            pltpu.VMEM((2, 2, D, FC), BF16),
            pltpu.VMEM((F, D), BF16),
            pltpu.VMEM((N_PROD, ROWS // 2, D // 4), U32),
            pltpu.VMEM((S // ROWS, D // LANES, ROWS + PAD, LANES), F32),
            pltpu.SMEM((1,), jnp.int32),
            pltpu.SemaphoreType.DMA((len(_WAITS),)),
            pltpu.SemaphoreType.DMA((2,)),
            pltpu.SemaphoreType.DMA(()),
            pltpu.SemaphoreType.DMA(()),
        ],
        compiler_params=pltpu.CompilerParams(vmem_limit_bytes=127 * 2**20),
    )(A_x.reshape(S, D), A_wqkv, A_wo, B_w_gate, B_w_up, B_w_down)
    return out.reshape(B, S, D)
```
